```python
import os as _os
_os.environ.setdefault("JAX_PLATFORMS", "cpu")
import jax
import jax.numpy as jnp

def _softmax(x, axis=-1):
    return jax.nn.softmax(x, axis=axis)
def _gelu(x):
    return jax.nn.gelu(x, approximate=True)
def _silu(x):
    return jax.nn.silu(x)
def _sigmoid(x):
    return jax.nn.sigmoid(x)
def _layernorm(x, axis=-1, eps=1e-5):
    m = jnp.mean(x, axis=axis, keepdims=True)
    v = jnp.var(x, axis=axis, keepdims=True)
    return (x - m) / jnp.sqrt(v + eps)
def _scatter_add(tgt, idx, src, axis=0):
    return tgt.at[idx].add(src)
def _segment_sum(src, seg, n):
    return jax.ops.segment_sum(src, seg, n)
class _Rng:
    def __init__(self, key):
        self._k = key
    def _next(self):
        self._k, sub = jax.random.split(self._k)
        return sub
    def normal(self, shape):
        return jax.random.normal(self._next(), shape, dtype=jnp.bfloat16)
    def randint(self, lo, hi, shape):
        return jax.random.randint(self._next(), shape, lo, hi, dtype=jnp.int32)
    def uniform(self, shape, lo=0.0, hi=1.0):
        return jax.random.uniform(self._next(), shape, jnp.bfloat16, lo, hi)
    def permutation(self, n):
        return jax.random.permutation(self._next(), n)


kernel_name = 'concat_heads__mha_block__ssm_conv_s4__prompt'

def setup_inputs():
    _rng = _Rng(jax.random.key(int.from_bytes(__import__("os").urandom(4), "little")))
    _w = (lambda a: (lambda t: t.astype(jnp.bfloat16) if jnp.issubdtype(t.dtype, jnp.floating) else t)(jnp.asarray(a)))
    def _A_setup():
        B, S, D, H = 1, 2048, 448, 16
        return {
            "x": _w((lambda *s: _rng.normal(s) * 0.2)(B, S, D)),
            "wqkv": _w((lambda *s: _rng.normal(s) * 0.2)(D, 3 * D)),
            "wo": _w((lambda *s: _rng.normal(s) * 0.05)(D, D)),
        }
    _A_in = _A_setup()

    def _B_setup():
        B, L, D, N = 1, 2048, 448, 256
        A_re = -jnp.exp((lambda *s: _rng.normal(s) * 0.2)(D, N))
        A_im = jnp.pi * (lambda *s: _rng.normal(s) * 0.2)(D, N)
        B_re = (lambda *s: _rng.normal(s) * 0.2)(D, N)
        B_im = (lambda *s: _rng.normal(s) * 0.2)(D, N)
        C_re = (lambda *s: _rng.normal(s) * 0.2)(D, N)
        C_im = (lambda *s: _rng.normal(s) * 0.2)(D, N)
        log_dt = (lambda *s: _rng.normal(s) * 0.2)(D) * 0.5 - 4.0
        Dskip = (lambda *s: _rng.normal(s) * 0.05)(D)
        return {
            "u": _w((lambda *s: _rng.normal(s) * 0.05)(B, L, D)),
            "A_re": _w(A_re),
            "A_im": _w(A_im),
            "B_re": _w(B_re),
            "B_im": _w(B_im),
            "C_re": _w(C_re),
            "C_im": _w(C_im),
            "log_dt": _w(log_dt),
            "Dskip": _w(Dskip),
        }
    _B_in = _B_setup()

    return {
        "A_x": _A_in["x"],
        "A_wqkv": _A_in["wqkv"],
        "A_wo": _A_in["wo"],
        "B_u": _B_in["u"],
        "B_A_re": _B_in["A_re"],
        "B_A_im": _B_in["A_im"],
        "B_B_re": _B_in["B_re"],
        "B_B_im": _B_in["B_im"],
        "B_C_re": _B_in["C_re"],
        "B_C_im": _B_in["C_im"],
        "B_log_dt": _B_in["log_dt"],
        "B_Dskip": _B_in["Dskip"],
    }

def reference(A_x, A_wqkv, A_wo, B_u, B_A_re, B_A_im, B_B_re, B_B_im, B_C_re, B_C_im, B_log_dt, B_Dskip):
    def _A_ref(x, wqkv, wo):
        B, S, D = x.shape
        H = 16
        Dh = D // H
        qkv = (lambda x, *d: x.transpose(*d))((x @ wqkv).reshape(B, S, 3, H, Dh), 2, 0, 3, 1, 4)
        q, k, v = qkv[0], qkv[1], qkv[2]
        scores = jnp.einsum("bhqd,bhkd->bhqk", q, k) * (Dh ** -0.5)
        p = _softmax(scores, axis=-1)
        o = jnp.einsum("bhqk,bhkd->bhqd", p, v)
        return (lambda x, *d: x.transpose(*d))(o, 0, 2, 1, 3).reshape(B, S, D) @ wo

    def _B_ref(u, A_re, A_im, B_re, B_im, C_re, C_im, log_dt, Dskip):
        Bsz, L, D = u.shape
        dt = jnp.exp(log_dt)[:, None]
        A = A_re + 1j * A_im
        Bc = B_re + 1j * B_im
        Cc = C_re + 1j * C_im
        logdA = dt * A
        dB = dt * Bc
        l = (lambda x, dt: x.astype(dt))(jnp.arange(L), A_re.dtype)
        P = jnp.exp(logdA[:, :, None] * l[None, None, :])
        K = jnp.einsum("dn,dnl,dn->dl", Cc, P, dB).real
        L2 = 2 * L
        Kp = jnp.pad(K, ((0, 0), (0, L)))
        up = (lambda x, *d: x.transpose(*d))(u, 0, 2, 1)
        up = jnp.pad(up, ((0, 0), (0, 0), (0, L)))
        Kf = (lambda x, axes=(-2,-1): jnp.fft.rfft2(x.astype(jnp.float32), axes=axes))(Kp[:, None, :], axes=(-2, -1))
        Uf = (lambda x, axes=(-2,-1): jnp.fft.rfft2(x.astype(jnp.float32), axes=axes))(up[:, :, None, :], axes=(-2, -1))
        Yf = Uf * Kf[None, :, :, :]
        y = (lambda x, s, axes=(-2,-1): jnp.fft.irfft2(x, s=s, axes=axes).astype(jnp.bfloat16))(Yf, (1, L2), axes=(-2, -1))[:, :, 0, :L]
        y = (lambda x, *d: x.transpose(*d))(y, 0, 2, 1) + u * Dskip[None, None, :]
        return y

    a = _A_ref(A_x, A_wqkv, A_wo)
    b = _B_ref(B_u, B_A_re, B_A_im, B_B_re, B_B_im, B_C_re, B_C_im, B_log_dt, B_Dskip)
    return jnp.concatenate([a, b], axis=-1)
```

```python
import functools, contextlib
import numpy as np
import jax
import jax.numpy as jnp
from jax import lax
import jax.experimental.pallas as pl
import jax.experimental.pallas.tpu as pltpu
import ml_dtypes

S, D, H, DH, N = 2048, 448, 16, 28, 256
NQ = 512
R = 128
SL = 32
NSL = D // SL
NCB = 4
CB = S // NCB
NT = (((1,), (1,)), ((), ()))
TN = (((0,), (0,)), ((), ()))
f32, bf16, i32 = jnp.float32, jnp.bfloat16, jnp.int32
LOG2E = 1.4426950408889634

def _rbf16(l):
    x = np.asarray(l, np.float32)
    u = x.view(np.uint32).astype(np.uint64)
    u = (u + 0x7FFF + ((u >> 16) & 1)) & 0xFFFF0000
    return u.astype(np.uint32).view(np.float32).astype(np.float64)

HI = np.array([0, 1, 2, 3, 4, 5, 6, 7, 512, 516, 1024, 1536, 640, 1152, 1664, 0])

def dft_consts():
    T, M = 128, 256
    forder = np.concatenate([np.arange(0, 128, 2), np.arange(1, 128, 2)])
    ang = 2 * np.pi * (forder[:, None] + 0.5) * np.arange(T)[None, :] / M
    F = np.concatenate([np.cos(ang), -np.sin(ang)], 0)
    Finv = np.concatenate([np.cos(ang).T, -np.sin(ang).T], 1) * (2.0 / M)
    def lag_of(upper, blk):
        r = np.arange(8)[:, None] + (8 if upper else 0)
        b = 16 * blk + np.arange(16)[None, :]
        return (HI[r] + 8 * b).reshape(-1)
    plan = []
    Gs = []
    for m in range(16):
        tgt = _rbf16(128 * m + np.arange(T)).astype(int)
        if m < 4: cand = [(0, m)] + ([(0, m + 1)] if m == 2 else []) + ([(1, 0)] if m == 3 else [])
        elif m < 8: cand = [(1, m - 4)]
        elif m < 12: cand = [(1, m - 8)]
        else: cand = [(1, m - 12)]
        used = np.zeros(T, bool)
        for (up, blk) in cand:
            lg = lag_of(up, blk)
            valid = np.ones(128, bool)
            if up: valid[7 * 16:] = False
            E = np.zeros((T, 128))
            for j in range(T):
                if used[j]: continue
                idx = np.where((lg == tgt[j]) & valid)[0]
                if len(idx):
                    E[j, idx[0]] = 1; used[j] = True
            Gm = F @ E
            gi = None
            for k, g0 in enumerate(Gs):
                if np.array_equal(g0, Gm): gi = k
            if gi is None:
                Gs.append(Gm); gi = len(Gs) - 1
            plan.append((m, up, blk, gi))
        assert used.all()
    return F, Finv, np.stack(Gs), plan


_F, _FINV, _G, _PLAN = dft_consts()
_bf = lambda a: np.asarray(a, np.float32).astype(ml_dtypes.bfloat16)
C_FT = _bf(_F.T)
C_FINVT = _bf(_FINV.T)
C_GT = _bf(np.transpose(_G, (0, 2, 1)))
FLAGS = {}
_KNOBS = {'SP0': '1.1', 'SP1': '1.15', 'MAXMM': '2', 'BR': '1', 'MM': '11', 'GSPL': '1', 'TPRO': '0', 'LAYOUT': 'a'}
E = _KNOBS.get
CFG = dict(g3=E("G3", "1") == "1", layout=E("LAYOUT", "a"), sep=E("SEP", "0") == "1")
pk = lambda x: pltpu.bitcast(x, i32)
upk = lambda x: pltpu.bitcast(x, bf16)


def cmul(ar, ai, br, bi):
    return ar * br - ai * bi, ar * bi + ai * br


def fold8(t):
    sub = lax.broadcasted_iota(jnp.int32, (8, 128), 0)
    seg = lax.broadcasted_iota(jnp.int32, (8, 128), 1) >> 4
    for k in (4, 2, 1):
        sb = (sub & k) != 0
        gb = (seg & k) != 0
        up = pltpu.roll(pltpu.roll(t, 8 - k, 0), 16 * k, 1)
        dn = pltpu.roll(pltpu.roll(t, k, 0), 128 - 16 * k, 1)
        t = jnp.where(sb == gb, t, jnp.where(gb, up, dn))
    return t


def sub_transpose8(xs):
    xs = list(xs)
    sub = lax.broadcasted_iota(jnp.int32, (8, 128), 0)
    for k in (4, 2, 1):
        keep = (sub & k) == 0
        new = list(xs)
        for a in range(8):
            if a & k:
                continue
            b = a ^ k
            new[a] = jnp.where(keep, xs[a], pltpu.roll(xs[b], k, 0))
            new[b] = jnp.where(keep, pltpu.roll(xs[a], 8 - k, 0), xs[b])
        xs = new
    return xs


def sel_matrix(rows0, nrows, col0, ncols, off):
    p = rows0 + lax.broadcasted_iota(jnp.int32, (nrows, ncols), 0)
    c = col0 + lax.broadcasted_iota(jnp.int32, (nrows, ncols), 1)
    j = p & 31
    src = off + 28 * (p >> 5) + j
    return jnp.where((src == c) & (j < 28), 1.0, 0.0).astype(bf16)


class Pump:
    def __init__(self, gen, total):
        self.gen, self.total, self.done = gen, total, 0.0
        self.pending = next(gen, None) if gen is not None else None
    def to(self, frac, mm=True, max_mm=99):
        n_mm = 0
        while self.pending is not None and self.done < frac * self.total - 1e-9:
            kind, cost = self.pending
            if kind == "m":
                if not mm or n_mm >= max_mm:
                    break
                n_mm += 1
            self.done += cost
            self.pending = next(self.gen, None)
    def finish(self):
        while self.pending is not None:
            self.pending = next(self.gen, None)


def chain(*gens):
    for g_ in gens:
        yield from g_


def kernel(z_ref, xt_hbm, wqkv_hbm, wo_hbm, ut_hbm, are_hbm, aim_hbm, bre_hbm, bim_hbm, cre_hbm, cim_hbm, ldt_ref, dsk_ref,
           FT_hbm, FinvT_hbm, GT_hbm,
           out_hbm,
           xt_ref, wqkv_ref, wo_ref, uin_ref, par_ref, FT_ref, FinvT_ref, GT_ref, ost_ref,
           wt_ref, wp_ref, wop_ref, qm_ref, k_ref, vt_ref, sA, sB, mA, mB, ot_ref,
           col_ref, a_tab, v0_tab, y8_tab, kt_ref, bm_ref, ut_ref, yt_ref, yh_ref, sem_in, sem_out):
    SC = (lambda n: jax.named_scope(n)) if False else (lambda n: contextlib.nullcontext())
    zz = z_ref[0]
    GSPL = E("GSPL", "1") == "1"
    TPRO = E("TPRO", "0") == "1"
    par_hbm = (are_hbm, aim_hbm, bre_hbm, bim_hbm, cre_hbm, cim_hbm)
    WOFF = ((384, 512), (896, 448), (0, 512))
    cp_w = [pltpu.make_async_copy(wqkv_hbm.at[:, pl.ds(a, n)], wqkv_ref.at[:, pl.ds(a, n)], sem_in.at[k])
            for k, (a, n) in enumerate(((384, 512), (896, 448), (0, 384)))]
    cp_x = [pltpu.make_async_copy(xt_hbm.at[:, pl.ds(cb * CB, CB)], xt_ref.at[:, pl.ds(cb * CB, CB)], sem_in.at[3 + cb]) for cb in range(NCB)]
    cp_p = [pltpu.make_async_copy(par_hbm[k], par_ref.at[k], sem_in.at[7 + k]) for k in range(6)]
    cp_wo = pltpu.make_async_copy(wo_hbm, wo_ref, sem_in.at[13])
    cp_c = [pltpu.make_async_copy(a, b, sem_in.at[14 + k]) for k, (a, b) in
            enumerate(((FT_hbm, FT_ref), (FinvT_hbm, FinvT_ref), (GT_hbm, GT_ref)))]
    cp_u = pltpu.make_async_copy(ut_hbm, uin_ref, sem_in.at[17])
    for cp in [cp_w[0], cp_x[0], cp_w[1], cp_w[2]] + cp_x[1:] + cp_p + [cp_wo] + cp_c + [cp_u]:
        cp.start()

    yt_ref[0:64, :] = jnp.zeros((64, S), bf16)
    yh_ref[...] = jnp.zeros(yh_ref.shape, f32)
    ldt = ldt_ref[...].astype(f32).reshape(1, D)
    dsk = dsk_ref[...].astype(f32).reshape(1, D)
    dt_row = jnp.exp(ldt).astype(bf16).astype(f32)
    col_ref[0] = jnp.broadcast_to(dt_row, (128, D)).T
    col_ref[1] = jnp.broadcast_to(dsk, (128, D)).T

    def w_transpose(tiles):
        for c in tiles:
            c1 = min(128 * (c + 1), 3 * D)
            blk = wqkv_ref[:, 128 * c:c1]
            blk = jnp.concatenate([blk, jnp.zeros((512 - D, c1 - 128 * c), bf16)], axis=0)
            if c1 - 128 * c < 128:
                blk = jnp.concatenate([blk, jnp.zeros((512, 128 - (c1 - 128 * c)), bf16)], axis=1)
            wt_ref[64 * c:64 * (c + 1), :] = pk(blk.T)
    def w_respace(part):
        z2 = jnp.zeros((2, 512), i32)
        for h in range(16):
            r0 = (D * part + DH * h) // 2
            wp_ref[part, 16 * h:16 * (h + 1), :] = jnp.concatenate([wt_ref[r0:r0 + 14, :], z2], axis=0)

    def b_tables(s, v_lo, v_hi):
        s = jnp.minimum(s, NSL - 1)
        d0 = pl.multiple_of(s * SL, SL)
        if TPRO:
            trow = lambda v, c_: pl.ds(pl.multiple_of(8 * (d0 + 8 * v + c_), 8), 8)
            yrow = lambda v: pl.ds(pl.multiple_of(d0 + 8 * v, 8), 8)
        else:
            trow = lambda v, c_: slice((8 * v + c_) * 8, (8 * v + c_) * 8 + 8)
            yrow = lambda v: slice(8 * v, 8 * v + 8)
        for v in range(v_lo, v_hi):
            rs = pl.ds(pl.multiple_of(d0 + 8 * v, 8), 8)
            dt = col_ref[0, rs, :]
            for t in range(2):
                ls = slice(128 * t, 128 * (t + 1))
                ld = lambda k: par_ref[k, rs, ls].astype(f32)
                yield "v", 100
                a_re, a_im = dt * ld(0), dt * ld(1)
                mag = jnp.exp(a_re)
                zr = mag * jnp.cos(a_im)
                yield "v", 60
                z = (zr, mag * jnp.sin(a_im))
                yield "v", 60
                z2 = cmul(*z, *z)
                z4 = cmul(*z2, *z2)
                y = cmul(*z4, *z4)
                rows_ = [(jnp.ones_like(zr), jnp.zeros_like(zr)), y]
                for r in range(6):
                    rows_.append(cmul(*rows_[-1], *y))
                yield "v", 70
                tr = sub_transpose8([x_[0] for x_ in rows_])
                for c_ in range(8):
                    v0_tab[t, trow(v, c_), :] = tr[c_]
                yield "v", 70
                ti = sub_transpose8([x_[1] for x_ in rows_])
                for c_ in range(8):
                    v0_tab[2 + t, trow(v, c_), :] = ti[c_]
                yield "v", 40
                z16 = cmul(*y, *y)
                z32 = cmul(*z16, *z16)
                z64 = cmul(*z32, *z32)
                y8_tab[t, yrow(v), :] = z64[0]
                y8_tab[2 + t, yrow(v), :] = z64[1]
                z128 = cmul(*z64, *z64)
                z256 = cmul(*z128, *z128)
                z512 = cmul(*z256, *z256)
                yield "v", 60
                w = cmul(ld(4), ld(5), dt * ld(2), dt * ld(3))
                rows_ = [w]
                for r in range(7):
                    rows_.append(cmul(*rows_[-1], *z))
                yield "v", 50
                w512 = cmul(*w, *z512)
                w1024 = cmul(*w512, *z512)
                w1536 = cmul(*w1024, *z512)
                zero = jnp.zeros_like(zr)
                rows_ += [w512, cmul(*w512, *z4), w1024, w1536,
                          cmul(*w512, *z128), cmul(*w1024, *z128), cmul(*w1536, *z128), (zero, zero)]
                yield "v", 80
                pe = lambda a, b: pltpu.pack_elementwise([a, b], packed_dtype=bf16)
                wr = sub_transpose8([pe(rows_[2 * j][0], rows_[2 * j + 1][0]) for j in range(8)])
                for c_ in range(8):
                    a_tab[t, trow(v, c_), :] = wr[c_]
                yield "v", 90
                wi = sub_transpose8([pe(-rows_[2 * j][1], -rows_[2 * j + 1][1]) for j in range(8)])
                for c_ in range(8):
                    a_tab[2 + t, trow(v, c_), :] = wi[c_]
    T_OCT = 2 * 680

    scale = (DH ** -0.5) * LOG2E
    tpump = [None]
    def proj(part, cb):
        c0 = cb * CB
        xt = xt_ref[:, c0:c0 + CB]
        rows = lax.broadcasted_iota(jnp.int32, (128, CB), 0)
        for g in range(4):
            o_ = jnp.dot(upk(wp_ref[part, 64 * g:64 * (g + 1), :])[:, 0:D], xt, preferred_element_type=f32)
            if part == 1:
                k_ref[g, c0 // 2:(c0 + CB) // 2, :] = pk(o_.astype(bf16).T)
            elif part == 2:
                vt_ref[64 * g:64 * (g + 1), c0:c0 + CB] = pk(jnp.where((rows & 31) == 28, 1.0, o_).astype(bf16))
            else:
                q = o_ * scale
                for hh in range(4):
                    qm_ref[4 * g + hh, :, c0:c0 + CB] = pk(jnp.where((rows >> 5) == hh, q, 0.0).astype(bf16))
            if tpump[0] is not None:
                tcount[0] += 1
                tpump[0].to(tcount[0] / 36)
    with SC('wait_w'):
        cp_w[0].wait()
    w_transpose((3, 4, 5, 6))
    w_respace(1)
    cp_x[0].wait()
    proj(1, 0)
    cp_w[1].wait()
    cp_w[2].wait()
    w_transpose((7, 8, 9, 10, 0, 1, 2))
    w_respace(2)
    w_respace(0)
    proj(2, 0)
    proj(0, 0)
    if TPRO:
        for cp in cp_p:
            cp.wait()
        tcount = [0]
        tpump[0] = Pump(chain(*[b_tables(s_, 0, 4) for s_ in range(NSL)]), NSL * 4 * T_OCT)
    cp_x[1].wait()
    for part in (1, 2, 0):
        proj(part, 1)
    cp_x[2].wait()
    cp_x[3].wait()
    cp_wo.wait()
    wo = pk(wo_ref[...])
    z2 = jnp.zeros((2, D), i32)
    for h in range(16):
        wop_ref[16 * h:16 * (h + 1), :] = jnp.concatenate([wo[14 * h:14 * h + 14], z2], axis=0)
    for cb in range(2, NCB):
        for part in (1, 2, 0):
            proj(part, cb)
    if TPRO:
        tpump[0].finish()
    for cp in ([] if TPRO else cp_p) + cp_c + [cp_u]:
        cp.wait()

    def b_inv(s):
        r0 = pl.multiple_of(64 + s * SL, SL)
        for ib in range(4):
            yield "m", 100
            lhs = yh_ref[4 * SL * ib:4 * SL * (ib + 1), :].astype(bf16)
            o = jnp.dot(lhs, FinvT_ref[...], preferred_element_type=f32)
            for k in range(4):
                i = 4 * ib + k
                yt_ref[pl.ds(r0, SL), 128 * i:128 * (i + 1)] = o[k * SL:(k + 1) * SL].astype(bf16)

    def b_kgen(s, g_lo, g_hi):
        lane = lax.broadcasted_iota(jnp.int32, (8, 128), 1)
        HP = SL // 2
        if TPRO:
            d0 = pl.multiple_of(jnp.minimum(s, NSL - 1) * SL, SL)
        for g in range(g_lo, g_hi):
            def row(d, n):
                if TPRO:
                    return pl.ds(pl.multiple_of(8 * (d0 + d), 8), 8) if n == 8 else pl.ds(d0 + d, 1)
                return slice(8 * d, 8 * d + 8) if n == 8 else slice(d, d + 1)
            if not GSPL:
                rhs = [[None] * 2 for _ in range(4)]
                lhs = [[None] * 2 for _ in range(4)]
                for ch in range(2):
                    d = g + HP * ch
                    for t in range(2):
                        yield "v", 50
                        vr, vi = v0_tab[t, row(d, 8), :], v0_tab[2 + t, row(d, 8), :]
                        mr = jnp.broadcast_to(y8_tab[t, row(d, 1), :], (8, 128))
                        mi = jnp.broadcast_to(y8_tab[2 + t, row(d, 1), :], (8, 128))
                        rr, ii = [vr], [vi]
                        for j in range(7):
                            nr, ni = cmul(rr[-1], ii[-1], mr, mi)
                            rr.append(nr); ii.append(ni)
                        rhs[t][ch] = jnp.concatenate(rr, axis=0)
                        rhs[2 + t][ch] = jnp.concatenate(ii, axis=0)
                    for t in range(4):
                        lhs[t][ch] = upk(a_tab[t, row(d, 8), :])
                yield "m", 40
                A = jnp.concatenate([jnp.concatenate([lhs[t][0], lhs[t][1]], axis=0) for t in range(4)], axis=1)
                Bm = jnp.concatenate([jnp.concatenate([rhs[t][0], rhs[t][1]], axis=0) for t in range(4)], axis=1).astype(bf16)
                o = lax.dot_general(A, Bm, NT, preferred_element_type=f32)
            else:
                o = None
                for t in range(2):
                    re_, im_ = [], []
                    for ch in range(2):
                        d = g + HP * ch
                        yield "v", 50
                        vr, vi = v0_tab[t, row(d, 8), :], v0_tab[2 + t, row(d, 8), :]
                        mr = jnp.broadcast_to(y8_tab[t, row(d, 1), :], (8, 128))
                        mi = jnp.broadcast_to(y8_tab[2 + t, row(d, 1), :], (8, 128))
                        rr, ii = [vr], [vi]
                        for j in range(7):
                            nr, ni = cmul(rr[-1], ii[-1], mr, mi)
                            rr.append(nr); ii.append(ni)
                        re_.extend(rr)
                        im_.extend(ii)
                    yield "m", 20
                    for kt_, rhs in ((t, re_), (2 + t, im_)):
                        A = jnp.concatenate([upk(a_tab[kt_, row(g + HP * ch, 8), :]) for ch in range(2)], axis=0)
                        d_ = lax.dot_general(A, jnp.concatenate(rhs, axis=0).astype(bf16), NT, preferred_element_type=f32)
                        o = d_ if o is None else o + d_
            yield "v", 40
            t_lo = jnp.where(lane < 64, o[0:8], o[16:24])
            t_hi = jnp.where(lane < 64, o[8:16], o[24:32])
            kt_ref[0, 8 * g:8 * (g + 1), :] = fold8(t_lo)
            kt_ref[1, 8 * g:8 * (g + 1), :] = fold8(t_hi)
    G_PAIR = 280

    G3 = CFG["g3"]
    def put_bu(ref, j, vr, vi, is_b):
        if not G3:
            ref[j, :, 0:128] = vr
            ref[j, :, 128:256] = vi
        elif is_b:
            ref[j, :, 0:128] = vr
            ref[j, :, 128:256] = vi - vr
            ref[j, :, 256:384] = vr + vi
        else:
            ref[j, :, 0:128] = vr + vi
            ref[j, :, 128:256] = vr
            ref[j, :, 256:384] = vi

    def b_dft(s):
        s = jnp.minimum(s, NSL - 1)
        d0 = pl.multiple_of(s * SL, SL)
        HP = SL // 2
        prev = None
        sgn = jnp.where(lax.broadcasted_iota(jnp.int32, (SL, 128), 1) < 64, 1.0, -1.0)
        for jb in range(4):
            yield "m", 120
            lhs = jnp.concatenate([uin_ref[pl.ds(d0, SL), 128 * j:128 * (j + 1)] for j in range(4 * jb, 4 * jb + 4)], axis=0)
            o = jnp.dot(lhs, FT_ref[...], preferred_element_type=f32)
            for k in range(4):
                j = 4 * jb + k
                ur, ui = o[k * SL:(k + 1) * SL, 0:128], o[k * SL:(k + 1) * SL, 128:256]
                if prev is None:
                    put_bu(ut_ref, j, ur, ui, False)
                else:
                    put_bu(ut_ref, j, ur - sgn * prev[1], ui + sgn * prev[0], False)
                prev = (ur, ui)
        tiles = {}
        for up in range(2):
            yield "v", 150
            for blk in range(4):
                parts = [kt_ref[up, pl.ds(ch * 4 + blk, HP, stride=8), :] for ch in range(2)]
                tiles[(up, blk)] = jnp.concatenate(parts, axis=0).astype(bf16)
        by_g = {}
        for (m, up, blk, gi) in _PLAN:
            by_g.setdefault(gi, []).append((m, up, blk))
        res = {}
        dcol = col_ref[1, pl.ds(d0, SL), :]
        for gi in range(6):
            yield "m", 120
            lst = by_g[gi]
            lhs = jnp.concatenate([tiles[(up, blk)] for (_, up, blk) in lst], axis=0)
            o = jnp.dot(lhs, GT_ref[gi], preferred_element_type=f32)
            for k, (m, _, _) in enumerate(lst):
                piece = o[k * SL:(k + 1) * SL]
                res[m] = piece if m not in res else res[m] + piece
            for m in sorted(set(x_[0] for x_ in lst)):
                if gi == 1:
                    continue
                vr, vi = res[m][:, 0:128], res[m][:, 128:256]
                if m == 0:
                    vr = vr + dcol
                put_bu(bm_ref, m, vr, vi, True)

    def b_conv(i_lo, i_hi):
        for i in range(i_lo, i_hi):
            for v in range(SL // 8):
                rs = slice(8 * v, 8 * (v + 1))
                a1 = a2 = a3 = None
                for m in range(i + 1):
                    if m % 2 == 0:
                        yield "v", 8 * min(2, i + 1 - m)
                    j = i - m
                    if G3:
                        p1 = bm_ref[m, rs, 0:128] * ut_ref[j, rs, 0:128]
                        p2 = bm_ref[m, rs, 128:256] * ut_ref[j, rs, 128:256]
                        p3 = bm_ref[m, rs, 256:384] * ut_ref[j, rs, 256:384]
                        a3 = p3 if a3 is None else a3 + p3
                    else:
                        p1, p2 = cmul(bm_ref[m, rs, 0:128], bm_ref[m, rs, 128:256], ut_ref[j, rs, 0:128], ut_ref[j, rs, 128:256])
                    a1 = p1 if a1 is None else a1 + p1
                    a2 = p2 if a2 is None else a2 + p2
                if G3:
                    yr, yi = a1 - a3, a1 + a2
                else:
                    yr, yi = a1, a2
                yh_ref[i * SL + 8 * v:i * SL + 8 * (v + 1), 0:128] = yr
                yh_ref[i * SL + 8 * v:i * SL + 8 * (v + 1), 128:256] = yi
    conv_cost = lambda a, b: sum(32 * (i + 1) for i in range(a, b))

    LAY = CFG["layout"]
    MAXMM = int(E("MAXMM", "1"))
    MM1, MM2 = E("MM", "10")[0] == "1", E("MM", "10")[1] == "1"
    def b_step(k, s):
        if LAY == "a":
            if k == 0:
                return chain(b_inv(s - 1), b_tables(s, 0, 4)), 4 * T_OCT + 400
            if k == 1:
                return b_kgen(s, 0, 16), 16 * G_PAIR
            if k == 2:
                return b_dft(s), 1500
            return b_conv(0, 16), conv_cost(0, 16)
        if LAY == "c":
            GS, CS = int(E("GS", "8")), int(E("CS", "12"))
            if k == 0:
                return chain(b_conv(CS, 16), b_kgen(s, 0, GS)), conv_cost(CS, 16) + GS * G_PAIR
            if k == 1:
                return chain(b_kgen(s, GS, 16)), (16 - GS) * G_PAIR
            if k == 2:
                return chain(b_inv(s - 1), b_dft(s)), 1900
            return b_conv(0, CS), conv_cost(0, CS)
        if LAY == "b":
            CS = 12
            if k == 0:
                return chain(b_conv(CS, 16), b_kgen(s, 0, 8)), conv_cost(CS, 16) + 8 * G_PAIR
            if k == 1:
                return chain(b_inv(s - 1), b_kgen(s, 8, 16)), 400 + 8 * G_PAIR
            if k == 2:
                return chain(b_dft(s), b_tables(s + 1, 0, 2)), 1500 + 2 * T_OCT
            return chain(b_tables(s + 1, 2, 4), b_conv(0, CS)), conv_cost(0, CS) + 2 * T_OCT

    def stage(i, s_new, m_new, s_old, m_old, do_q=True, do_e=True, bwork=None, speed=1.0):
        nchunk = S // R
        pump = Pump(*bwork) if bwork is not None else Pump(None, 0)
        if do_e:
            h = i % 16
            q0 = pl.multiple_of((i // 16) * NQ, NQ)
            r0 = pl.multiple_of(h * 16, 16)
            mo = jnp.max(m_old[...], axis=0, keepdims=True)
        if do_q:
            hq = (i + 1) % 16
            qq0 = pl.multiple_of((((i + 1) // 16) % 4) * NQ, NQ)
            h4 = hq // 4
            qm = upk(qm_ref[hq, :, pl.ds(qq0, NQ)])
        mrun = None
        acc = None
        for c in range(nchunk):
            rs = slice(c * R, (c + 1) * R)
            if do_q:
                s = jnp.dot(upk(k_ref[h4, c * R // 2:(c + 1) * R // 2, :]), qm, preferred_element_type=f32)
            if do_e:
                p = jnp.exp2(s_old[rs, :] - mo).astype(bf16)
            pump.to(speed * (2 * c + 1) / (2 * nchunk), mm=MM1, max_mm=MAXMM)
            if do_q:
                s_new[rs, :] = s
                mc = jnp.max(s.reshape(R // 8, 8, NQ), axis=0)
                mrun = mc if mrun is None else jnp.maximum(mrun, mc)
            if do_e:
                d_ = jnp.dot(upk(vt_ref[pl.ds(r0, 16), rs]), p, preferred_element_type=f32)
                acc = d_ if acc is None else acc + d_
            pump.to(speed * (2 * c + 2) / (2 * nchunk), mm=MM2, max_mm=MAXMM)
        pump.finish()
        if do_q:
            m_new[...] = mrun
        if do_e:
            o = acc / acc[28:29, :]
            ot_ref[pl.ds(pl.multiple_of(h * 32, 32), 32), pl.ds(q0, NQ)] = o.astype(bf16)

    def out_proj(qb):
        q0 = pl.multiple_of(qb * NQ, NQ)
        oa = lax.dot_general(ot_ref[:, pl.ds(q0, NQ)], upk(wop_ref[...]), TN, preferred_element_type=f32)
        ost_ref[pl.ds(q0, NQ), 0:448] = oa.astype(bf16)

    def finish_b():
        for tb in range(S // NQ):
            rs = slice(NQ * tb, NQ * (tb + 1))
            yb = yt_ref[:, rs].T
            ost_ref[rs, 448:896] = yb[:, 64:512]

    def out_copy(qb):
        return pltpu.make_async_copy(ost_ref.at[pl.ds(qb * NQ, NQ)], out_hbm.at[pl.ds(qb * NQ, NQ)], sem_out.at[qb])

    n_units = 16 * (S // NQ)
    sep = (lambda f: pl.when(zz == 0)(f)) if CFG["sep"] else (lambda f: f())
    def b_unit(i, k, s):
        bufs = (sB, mB, sA, mA) if k % 2 == 0 else (sA, mA, sB, mB)
        with SC(f'stageB{k}'):
            stage(i, *bufs, bwork=b_step(k, s), speed=float(E('SP%d' % k, '1.0')))

    if LAY == "b":
        Pump(b_tables(0, 0, 4), 1).finish()
    stage(-1, sA, mA, None, None, do_e=False)

    def body_s(i, c):
        s = i // 4
        for k in range(4):
            @pl.when(i % 4 == k)
            def _():
                b_unit(i, k, s)
        @pl.when(i % 16 == 15)
        def _():
            with SC('outproj'):
                out_proj(i // 16)
        return c
    def body_m(s, c):
        for k in range(4):
            b_unit(4 * s + k, k, s)
        @pl.when(s % 4 == 3)
        def _():
            with SC('outproj'):
                out_proj(s // 4)
        return c
    def body2(j, c):
        i = first2 + 2 * j
        bufs = ((sB, mB, sA, mA), (sA, mA, sB, mB))
        sep(lambda: stage(i, *bufs[first2 % 2]))
        sep(lambda: stage(i + 1, *bufs[(first2 + 1) % 2]))
        return c
    with SC('loop'):
        if E('BR', '1') == '1':
            lax.fori_loop(0, 4 * NSL, body_s, 0)
        else:
            lax.fori_loop(0, NSL, body_m, 0)
        if LAY == "a":
            sep(lambda: b_unit(4 * NSL, 0, NSL))
            first2 = 4 * NSL + 1
        elif LAY == "c":
            CS = int(E("CS", "12"))
            sep(lambda: stage(4 * NSL, sB, mB, sA, mA, bwork=(b_conv(CS, 16), conv_cost(CS, 16))))
            sep(lambda: stage(4 * NSL + 1, sA, mA, sB, mB, bwork=(b_inv(NSL - 1), 400)))
            first2 = 4 * NSL + 2
        else:
            sep(lambda: stage(4 * NSL, sB, mB, sA, mA, bwork=(b_conv(12, 16), conv_cost(12, 16))))
            sep(lambda: stage(4 * NSL + 1, sA, mA, sB, mB, bwork=(b_inv(NSL - 1), 400)))
            first2 = 4 * NSL + 2
        finish_b()
        for qb in range(3):
            out_copy(qb).start()
        n2 = (n_units - 1 - first2) // 2
        lax.fori_loop(0, n2, body2, 0)
        for i in range(first2 + 2 * n2, n_units - 1):
            sep(lambda: stage(i, *((sB, mB, sA, mA) if i % 2 == 0 else (sA, mA, sB, mB))))
        stage(n_units - 1, None, None, sB, mB, do_q=False)
        out_proj(3)
    with SC('tail'):
        out_copy(3).start()
        for qb in range(4):
            out_copy(qb).wait()


@jax.jit
def pallas_concat_heads__mha_block__ssm_conv_s4__prompt_kernel(A_x, A_wqkv, A_wo, B_u, B_A_re, B_A_im, B_B_re, B_B_im, B_C_re, B_C_im, B_log_dt, B_Dskip):
    V = pltpu.VMEM
    FW = 384 if CFG["g3"] else 256
    TD = D if E("TPRO", "0") == "1" else SL
    scratch = [
        V((D, S), bf16), V((D, 3 * D), bf16), V((D, D), bf16), V((D, S), bf16), V((6, D, N), bf16),
        V((128, 256), bf16), V((256, 128), bf16), V((6, 128, 256), bf16), V((S, 2 * D), bf16),
        V((704, 512), i32), V((3, 256, 512), i32), V((256, D), i32),
        V((16, 64, S), i32), V((4, S // 2, 128), i32), V((256, S), i32),
        V((S, NQ), f32), V((S, NQ), f32), V((8, NQ), f32), V((8, NQ), f32), V((512, S), bf16),
        V((2, D, 128), f32),
        V((4, 8 * TD, 128), i32), V((4, 8 * TD, 128), f32), V((4, TD, 128), f32),
        V((2, 8 * (SL // 2), 128), f32),
        V((16, SL, FW), f32), V((16, SL, FW), f32),
        V((512, S), bf16), V((16 * SL, 256), f32),
        pltpu.SemaphoreType.DMA((18,)), pltpu.SemaphoreType.DMA((4,)),
    ]
    anyspec = pl.BlockSpec(memory_space=pl.ANY)
    vspec = pl.BlockSpec(memory_space=pltpu.VMEM)
    out = pl.pallas_call(
        kernel,
        out_shape=jax.ShapeDtypeStruct((S, 2 * D), bf16),
        in_specs=[pl.BlockSpec(memory_space=pltpu.SMEM)] + [anyspec] * 10 + [vspec, vspec] + [anyspec] * 3,
        out_specs=anyspec,
        scratch_shapes=scratch,
        compiler_params=pltpu.CompilerParams(vmem_limit_bytes=124 * 1024 * 1024, flags=FLAGS or None),
    )(np.zeros((1,), np.int32), A_x.reshape(S, D).T, A_wqkv, A_wo, B_u.reshape(S, D).T, B_A_re, B_A_im, B_B_re, B_B_im, B_C_re, B_C_im, B_log_dt, B_Dskip,
      C_FT, C_FINVT, C_GT)
    return out.reshape(1, S, 2 * D)
```

```python
import functools, contextlib
import numpy as np
import jax
import jax.numpy as jnp
from jax import lax
import jax.experimental.pallas as pl
import jax.experimental.pallas.tpu as pltpu
import ml_dtypes

S, D, H, DH, N = 2048, 448, 16, 28, 256
NQ = 512
R = 128
SL = 32
NSL = D // SL
NCB = 4
CB = S // NCB
NT = (((1,), (1,)), ((), ()))
TN = (((0,), (0,)), ((), ()))
f32, bf16, i32 = jnp.float32, jnp.bfloat16, jnp.int32
LOG2E = 1.4426950408889634

def _rbf16(l):
    x = np.asarray(l, np.float32)
    u = x.view(np.uint32).astype(np.uint64)
    u = (u + 0x7FFF + ((u >> 16) & 1)) & 0xFFFF0000
    return u.astype(np.uint32).view(np.float32).astype(np.float64)

HI = np.array([0, 1, 2, 3, 4, 5, 6, 7, 512, 516, 1024, 1536, 640, 1152, 1664, 0])

def dft_consts():
    T, M = 128, 256
    forder = np.concatenate([np.arange(0, 128, 2), np.arange(1, 128, 2)])
    ang = 2 * np.pi * (forder[:, None] + 0.5) * np.arange(T)[None, :] / M
    F = np.concatenate([np.cos(ang), -np.sin(ang)], 0)
    Finv = np.concatenate([np.cos(ang).T, -np.sin(ang).T], 1) * (2.0 / M)
    def lag_of(upper, blk):
        r = np.arange(8)[:, None] + (8 if upper else 0)
        b = 16 * blk + np.arange(16)[None, :]
        return (HI[r] + 8 * b).reshape(-1)
    plan = []
    Gs = []
    for m in range(16):
        tgt = _rbf16(128 * m + np.arange(T)).astype(int)
        if m < 4: cand = [(0, m)] + ([(0, m + 1)] if m == 2 else []) + ([(1, 0)] if m == 3 else [])
        elif m < 8: cand = [(1, m - 4)]
        elif m < 12: cand = [(1, m - 8)]
        else: cand = [(1, m - 12)]
        used = np.zeros(T, bool)
        for (up, blk) in cand:
            lg = lag_of(up, blk)
            valid = np.ones(128, bool)
            if up: valid[7 * 16:] = False
            E = np.zeros((T, 128))
            for j in range(T):
                if used[j]: continue
                idx = np.where((lg == tgt[j]) & valid)[0]
                if len(idx):
                    E[j, idx[0]] = 1; used[j] = True
            Gm = F @ E
            gi = None
            for k, g0 in enumerate(Gs):
                if np.array_equal(g0, Gm): gi = k
            if gi is None:
                Gs.append(Gm); gi = len(Gs) - 1
            plan.append((m, up, blk, gi))
        assert used.all()
    return F, Finv, np.stack(Gs), plan


_F, _FINV, _G, _PLAN = dft_consts()
_bf = lambda a: np.asarray(a, np.float32).astype(ml_dtypes.bfloat16)
C_FT = _bf(_F.T)
C_FINVT = _bf(_FINV.T)
C_GT = _bf(np.transpose(_G, (0, 2, 1)))
FLAGS = {}
_KNOBS = {'TPRO': '0', 'LAYOUT': 'd', 'ONCE': '1', 'MIXA': '1', 'GSPL': '1', 'G3': '1', 'MIXB': '0', 'ORDB': 'FIT', 'SPB': '1.15', 'LASTEQ': '1', 'OPIN': '1', 'OPS': '100', 'SPA0': '1.2', 'SPA': '1.25', 'PORD': '1'}
E = _KNOBS.get
CFG = dict(g3=E("G3", "1") == "1", layout=E("LAYOUT", "a"), sep=E("SEP", "0") == "1")
pk = lambda x: pltpu.bitcast(x, i32)
upk = lambda x: pltpu.bitcast(x, bf16)


def cmul(ar, ai, br, bi):
    return ar * br - ai * bi, ar * bi + ai * br


def sincos(x):
    k = jnp.round(x * 0.6366197723675814)
    r = x - k * 1.5703125
    r = r - k * 4.837512969970703125e-4
    r = r - k * 7.54978995489188e-8
    r2 = r * r
    s = r + r * r2 * (-1.6666654611e-1 + r2 * (8.3321608736e-3 + r2 * -1.9515295891e-4))
    c = 1.0 + r2 * (-0.5 + r2 * (4.166664568298827e-2 + r2 * (-1.388731625493765e-3 + r2 * 2.443315711809948e-5)))
    q = k.astype(jnp.int32)
    swap = (q & 1) != 0
    s1 = jnp.where(swap, c, s)
    c1 = jnp.where(swap, s, c)
    s1 = jnp.where((q & 2) != 0, -s1, s1)
    c1 = jnp.where(((q + 1) & 2) != 0, -c1, c1)
    return s1, c1


def fold8(t):
    sub = lax.broadcasted_iota(jnp.int32, (8, 128), 0)
    seg = lax.broadcasted_iota(jnp.int32, (8, 128), 1) >> 4
    for k in (4, 2, 1):
        sb = (sub & k) != 0
        gb = (seg & k) != 0
        up = pltpu.roll(pltpu.roll(t, 8 - k, 0), 16 * k, 1)
        dn = pltpu.roll(pltpu.roll(t, k, 0), 128 - 16 * k, 1)
        t = jnp.where(sb == gb, t, jnp.where(gb, up, dn))
    return t


def sub_transpose8(xs):
    xs = list(xs)
    sub = lax.broadcasted_iota(jnp.int32, (8, 128), 0)
    for k in (4, 2, 1):
        keep = (sub & k) == 0
        new = list(xs)
        for a in range(8):
            if a & k:
                continue
            b = a ^ k
            new[a] = jnp.where(keep, xs[a], pltpu.roll(xs[b], k, 0))
            new[b] = jnp.where(keep, pltpu.roll(xs[a], 8 - k, 0), xs[b])
        xs = new
    return xs


def sel_matrix(rows0, nrows, col0, ncols, off):
    p = rows0 + lax.broadcasted_iota(jnp.int32, (nrows, ncols), 0)
    c = col0 + lax.broadcasted_iota(jnp.int32, (nrows, ncols), 1)
    j = p & 31
    src = off + 28 * (p >> 5) + j
    return jnp.where((src == c) & (j < 28), 1.0, 0.0).astype(bf16)


class Pump:
    def __init__(self, gen, total):
        self.gen, self.total, self.done = gen, total, 0.0
        self.pending = next(gen, None) if gen is not None else None
    def to(self, frac, mm=True, max_mm=99):
        n_mm = 0
        while self.pending is not None and self.done < frac * self.total - 1e-9:
            kind, cost = self.pending
            if kind == "m":
                if not mm or n_mm >= max_mm:
                    break
                n_mm += 1
            self.done += cost
            self.pending = next(self.gen, None)
    def finish(self):
        while self.pending is not None:
            self.pending = next(self.gen, None)


def chain(*gens):
    for g_ in gens:
        yield from g_


def mix(*items):
    st = [[g, float(t), 0.0, next(g, None)] for g, t in items]
    while True:
        live = [x for x in st if x[3] is not None]
        if not live:
            return
        x = min(live, key=lambda y: y[2] / y[1])
        kind, cost = x[3]
        yield kind, cost
        x[2] += cost
        x[3] = next(x[0], None)


def kernel(z_ref, xt_hbm, wqkv_hbm, wo_hbm, ut_hbm, are_hbm, aim_hbm, bre_hbm, bim_hbm, cre_hbm, cim_hbm, ldt_hbm, dsk_hbm,
           FT_hbm, FinvT_hbm, GT_hbm,
           out_hbm,
           ldt_ref, dsk_ref, xt_ref, wqkv_ref, wo_ref, uin_ref, par_ref, FT_ref, FinvT_ref, GT_ref, ost_ref,
           wt_ref, wp_ref, wop_ref, qm_ref, k_ref, vt_ref, sA, sB, mA, mB, ot_ref,
           col_ref, a_tab, v0_tab, y8_tab, kt_ref, bm_ref, ut_ref, yt_ref, yh_ref, opart_ref, sem_in, sem_out):
    SC = (lambda n: jax.named_scope(n)) if False else (lambda n: contextlib.nullcontext())
    zz = z_ref[0]
    LAY = CFG["layout"]
    GSPL = E("GSPL", "1") == "1"
    TPRO = E("TPRO", "0") == "1"
    par_hbm = (are_hbm, aim_hbm, bre_hbm, bim_hbm, cre_hbm, cim_hbm)
    WOFF = ((384, 512), (896, 448), (0, 512))
    cp_w = [pltpu.make_async_copy(wqkv_hbm.at[:, pl.ds(a, n)], wqkv_ref.at[:, pl.ds(a, n)], sem_in.at[k])
            for k, (a, n) in enumerate(((384, 512), (896, 448), (0, 384)))]
    cp_x = [pltpu.make_async_copy(xt_hbm.at[:, pl.ds(cb * CB, CB)], xt_ref.at[:, pl.ds(cb * CB, CB)], sem_in.at[3 + cb]) for cb in range(NCB)]
    cp_p = [pltpu.make_async_copy(par_hbm[k], par_ref.at[k], sem_in.at[7 + k]) for k in range(6)]
    cp_wo = pltpu.make_async_copy(wo_hbm, wo_ref, sem_in.at[13])
    cp_c = [pltpu.make_async_copy(a, b, sem_in.at[14 + k]) for k, (a, b) in
            enumerate(((FT_hbm, FT_ref), (FinvT_hbm, FinvT_ref), (GT_hbm, GT_ref)))]
    cp_u = pltpu.make_async_copy(ut_hbm, uin_ref, sem_in.at[17])
    cp_v = [pltpu.make_async_copy(ldt_hbm, ldt_ref, sem_in.at[18]), pltpu.make_async_copy(dsk_hbm, dsk_ref, sem_in.at[19])]
    for cp in ([cp_w[0], cp_x[0], cp_w[1], cp_w[2], cp_x[1]] if E('PORD', '0') == '0' else [cp_w[0], cp_x[0], cp_w[1], cp_x[1], cp_w[2]]) + cp_x[2:] + [cp_wo] + cp_v + cp_p + cp_c + [cp_u]:
        cp.start()

    yt_ref[0:64, :] = jnp.zeros((64, S), bf16)
    yh_ref[...] = jnp.zeros(yh_ref.shape, f32)
    def w_transpose(tiles):
        for c in tiles:
            c1 = min(128 * (c + 1), 3 * D)
            blk = wqkv_ref[:, 128 * c:c1]
            blk = jnp.concatenate([blk, jnp.zeros((512 - D, c1 - 128 * c), bf16)], axis=0)
            if c1 - 128 * c < 128:
                blk = jnp.concatenate([blk, jnp.zeros((512, 128 - (c1 - 128 * c)), bf16)], axis=1)
            wt_ref[64 * c:64 * (c + 1), :] = pk(blk.T)
    def w_respace(part, hs=range(16)):
        z2 = jnp.zeros((2, 512), i32)
        for h in hs:
            r0 = (D * part + DH * h) // 2
            wp_ref[part, 16 * h:16 * (h + 1), :] = jnp.concatenate([wt_ref[r0:r0 + 14, :], z2], axis=0)
    def w_prep_vq():
        for c in (7, 8, 9, 10, 0, 1, 2):
            yield "v", 2
            w_transpose((c,))
        for part in (2, 0):
            for h in range(0, 16, 4):
                yield "v", 1
                w_respace(part, range(h, h + 4))

    def b_tables(s, v_lo, v_hi):
        s = jnp.minimum(s, NSL - 1)
        d0 = pl.multiple_of(s * SL, SL)
        if TPRO:
            trow = lambda v, c_: pl.ds(pl.multiple_of(8 * (d0 + 8 * v + c_), 8), 8)
            yrow = lambda v: pl.ds(pl.multiple_of(d0 + 8 * v, 8), 8)
        else:
            trow = lambda v, c_: slice((8 * v + c_) * 8, (8 * v + c_) * 8 + 8)
            yrow = lambda v: slice(8 * v, 8 * v + 8)
        for v in range(v_lo, v_hi):
            rs = pl.ds(pl.multiple_of(d0 + 8 * v, 8), 8)
            dt = col_ref[0, rs, :]
            for t in range(2):
                ls = slice(128 * t, 128 * (t + 1))
                ld = lambda k: par_ref[k, rs, ls].astype(f32)
                yield "v", 100
                a_re, a_im = dt * ld(0), dt * ld(1)
                mag = jnp.exp(a_re)
                if E("SINCOS", "0") == "1":
                    sn, cs = sincos(a_im)
                    zr = mag * cs
                    z = (zr, mag * sn)
                else:
                    zr = mag * jnp.cos(a_im)
                    yield "v", 60
                    z = (zr, mag * jnp.sin(a_im))
                yield "v", 60
                z2 = cmul(*z, *z)
                z4 = cmul(*z2, *z2)
                y = cmul(*z4, *z4)
                rows_ = [(jnp.ones_like(zr), jnp.zeros_like(zr)), y]
                for r in range(6):
                    rows_.append(cmul(*rows_[-1], *y))
                yield "v", 70
                tr = sub_transpose8([x_[0] for x_ in rows_])
                for c_ in range(8):
                    v0_tab[t, trow(v, c_), :] = tr[c_]
                yield "v", 70
                ti = sub_transpose8([x_[1] for x_ in rows_])
                for c_ in range(8):
                    v0_tab[2 + t, trow(v, c_), :] = ti[c_]
                yield "v", 40
                z16 = cmul(*y, *y)
                z32 = cmul(*z16, *z16)
                z64 = cmul(*z32, *z32)
                y8_tab[t, yrow(v), :] = z64[0]
                y8_tab[2 + t, yrow(v), :] = z64[1]
                z128 = cmul(*z64, *z64)
                z256 = cmul(*z128, *z128)
                z512 = cmul(*z256, *z256)
                yield "v", 60
                w = cmul(ld(4), ld(5), dt * ld(2), dt * ld(3))
                rows_ = [w]
                for r in range(7):
                    rows_.append(cmul(*rows_[-1], *z))
                yield "v", 50
                w512 = cmul(*w, *z512)
                w1024 = cmul(*w512, *z512)
                w1536 = cmul(*w1024, *z512)
                zero = jnp.zeros_like(zr)
                rows_ += [w512, cmul(*w512, *z4), w1024, w1536,
                          cmul(*w512, *z128), cmul(*w1024, *z128), cmul(*w1536, *z128), (zero, zero)]
                yield "v", 80
                pe = lambda a, b: pltpu.pack_elementwise([a, b], packed_dtype=bf16)
                wr = sub_transpose8([pe(rows_[2 * j][0], rows_[2 * j + 1][0]) for j in range(8)])
                for c_ in range(8):
                    a_tab[t, trow(v, c_), :] = wr[c_]
                yield "v", 90
                wi = sub_transpose8([pe(-rows_[2 * j][1], -rows_[2 * j + 1][1]) for j in range(8)])
                for c_ in range(8):
                    a_tab[2 + t, trow(v, c_), :] = wi[c_]
    T_OCT = 2 * (620 if E("SINCOS", "0") == "1" else 680)

    scale = (DH ** -0.5) * LOG2E
    tpump = [None]
    tcount, tden = [0], [36]
    def proj(part, cb, gs=range(4)):
        c0 = cb * CB
        xt = xt_ref[:, c0:c0 + CB]
        rows = lax.broadcasted_iota(jnp.int32, (128, CB), 0)
        for g in gs:
            o_ = jnp.dot(upk(wp_ref[part, 64 * g:64 * (g + 1), :])[:, 0:D], xt, preferred_element_type=f32)
            if part == 1:
                k_ref[g, c0 // 2:(c0 + CB) // 2, :] = pk(o_.astype(bf16).T)
            elif part == 2:
                vt_ref[64 * g:64 * (g + 1), c0:c0 + CB] = pk(jnp.where((rows & 31) == 28, 1.0, o_).astype(bf16))
            else:
                q = o_ * scale
                for hh in range(4):
                    qm_ref[4 * g + hh, :, c0:c0 + CB] = pk(jnp.where((rows >> 5) == hh, q, 0.0).astype(bf16))
            if tpump[0] is not None:
                tcount[0] += 1
                tpump[0].to(tcount[0] / tden[0])
    with SC('wait_w'):
        cp_w[0].wait()
    w_transpose((3, 4, 5, 6))
    w_respace(1)
    with SC('wait_x0'):
        cp_x[0].wait()
    if E("PORD", "0") == "0":
        proj(1, 0)
        with SC('wait_wvq'):
            cp_w[1].wait()
            cp_w[2].wait()
            cp_x[1].wait()
        wpump = Pump(w_prep_vq(), 22)
        for g_ in range(4):
            wpump.to((g_ + 1) / 3 * 0.999)
            proj(1, 1, (g_,))
        wpump.finish()
        for part in (2, 0):
            for cb in range(2):
                proj(part, cb)
    else:
        def w_prep(tiles, part):
            for c in tiles:
                yield "v", 2
                w_transpose((c,))
            for h in range(0, 16, 4):
                yield "v", 1
                w_respace(part, range(h, h + 4))
        proj(1, 0, (0, 1, 2))
        with SC('wait_wv'):
            cp_w[1].wait()
        wpump = Pump(w_prep((7, 8, 9, 10), 2), 12)
        wpump.to(0.999)
        proj(1, 0, (3,))
        wpump.finish()
        proj(2, 0)
        with SC('wait_wvq'):
            cp_x[1].wait()
            cp_w[2].wait()
        wpump = Pump(w_prep((0, 1, 2), 0), 10)
        for g_ in range(4):
            wpump.to((g_ + 1) / 3 * 0.999)
            proj(1, 1, (g_,))
        wpump.finish()
        proj(2, 1)
        proj(0, 0)
        proj(0, 1)
    with SC('wait_x23'):
        cp_x[2].wait()
        cp_x[3].wait()
        cp_wo.wait()
        for cp in cp_v + cp_p:
            cp.wait()
    def late_prep():
        yield "v", 6
        ldt = ldt_ref[...].astype(f32).reshape(1, D)
        dsk = dsk_ref[...].astype(f32).reshape(1, D)
        dt_row = jnp.exp(ldt).astype(bf16).astype(f32)
        col_ref[0] = jnp.broadcast_to(dt_row, (128, D)).T
        col_ref[1] = jnp.broadcast_to(dsk, (128, D)).T
        wo = pk(wo_ref[...])
        z2 = jnp.zeros((2, D), i32)
        for h in range(16):
            if h % 4 == 0:
                yield "v", 1
            wop_ref[16 * h:16 * (h + 1), :] = jnp.concatenate([wo[14 * h:14 * h + 14], z2], axis=0)
    lpump = Pump(late_prep(), 10)
    for g_ in range(4):
        lpump.to((g_ + 1) / 3 * 0.999)
        proj(1, 2, (g_,))
    lpump.finish()
    if LAY in ("b", "d"):
        tden[0] = int(E("TDEN", "17"))
        tpump[0] = Pump(b_tables(0, 0, 4), 4 * T_OCT)
    for part, cb in ((2, 2), (0, 2), (1, 3), (2, 3), (0, 3)):
        proj(part, cb)
    if tpump[0] is not None:
        tpump[0].finish()

    def b_inv(s):
        r0 = pl.multiple_of(64 + s * SL, SL)
        for ib in range(4):
            yield "m", 100
            lhs = yh_ref[4 * SL * ib:4 * SL * (ib + 1), :].astype(bf16)
            o = jnp.dot(lhs, FinvT_ref[...], preferred_element_type=f32)
            for k in range(4):
                i = 4 * ib + k
                yt_ref[pl.ds(r0, SL), 128 * i:128 * (i + 1)] = o[k * SL:(k + 1) * SL].astype(bf16)

    def b_kgen(s, g_lo, g_hi):
        lane = lax.broadcasted_iota(jnp.int32, (8, 128), 1)
        HP = SL // 2
        if TPRO:
            d0 = pl.multiple_of(jnp.minimum(s, NSL - 1) * SL, SL)
        for g in range(g_lo, g_hi):
            def row(d, n):
                if TPRO:
                    return pl.ds(pl.multiple_of(8 * (d0 + d), 8), 8) if n == 8 else pl.ds(d0 + d, 1)
                return slice(8 * d, 8 * d + 8) if n == 8 else slice(d, d + 1)
            if not GSPL:
                rhs = [[None] * 2 for _ in range(4)]
                lhs = [[None] * 2 for _ in range(4)]
                for ch in range(2):
                    d = g + HP * ch
                    for t in range(2):
                        yield "v", 50
                        vr, vi = v0_tab[t, row(d, 8), :], v0_tab[2 + t, row(d, 8), :]
                        mr = jnp.broadcast_to(y8_tab[t, row(d, 1), :], (8, 128))
                        mi = jnp.broadcast_to(y8_tab[2 + t, row(d, 1), :], (8, 128))
                        rr, ii = [vr], [vi]
                        for j in range(7):
                            nr, ni = cmul(rr[-1], ii[-1], mr, mi)
                            rr.append(nr); ii.append(ni)
                        rhs[t][ch] = jnp.concatenate(rr, axis=0)
                        rhs[2 + t][ch] = jnp.concatenate(ii, axis=0)
                    for t in range(4):
                        lhs[t][ch] = upk(a_tab[t, row(d, 8), :])
                yield "m", 40
                A = jnp.concatenate([jnp.concatenate([lhs[t][0], lhs[t][1]], axis=0) for t in range(4)], axis=1)
                Bm = jnp.concatenate([jnp.concatenate([rhs[t][0], rhs[t][1]], axis=0) for t in range(4)], axis=1).astype(bf16)
                o = lax.dot_general(A, Bm, NT, preferred_element_type=f32)
            else:
                o = None
                for t in range(2):
                    re_, im_ = [], []
                    for ch in range(2):
                        d = g + HP * ch
                        yield "v", 50
                        vr, vi = v0_tab[t, row(d, 8), :], v0_tab[2 + t, row(d, 8), :]
                        mr = jnp.broadcast_to(y8_tab[t, row(d, 1), :], (8, 128))
                        mi = jnp.broadcast_to(y8_tab[2 + t, row(d, 1), :], (8, 128))
                        rr, ii = [vr], [vi]
                        for j in range(7):
                            nr, ni = cmul(rr[-1], ii[-1], mr, mi)
                            rr.append(nr); ii.append(ni)
                        re_.extend(rr)
                        im_.extend(ii)
                    yield "m", 20
                    for kt_, rhs in ((t, re_), (2 + t, im_)):
                        A = jnp.concatenate([upk(a_tab[kt_, row(g + HP * ch, 8), :]) for ch in range(2)], axis=0)
                        d_ = lax.dot_general(A, jnp.concatenate(rhs, axis=0).astype(bf16), NT, preferred_element_type=f32)
                        o = d_ if o is None else o + d_
            yield "v", 40
            t_lo = jnp.where(lane < 64, o[0:8], o[16:24])
            t_hi = jnp.where(lane < 64, o[8:16], o[24:32])
            kt_ref[0, 8 * g:8 * (g + 1), :] = fold8(t_lo)
            kt_ref[1, 8 * g:8 * (g + 1), :] = fold8(t_hi)
    G_PAIR = 280

    G3 = CFG["g3"]
    def put_bu(ref, j, vr, vi, is_b):
        if not G3:
            ref[j, :, 0:128] = vr
            ref[j, :, 128:256] = vi
        elif is_b:
            ref[j, :, 0:128] = vr
            ref[j, :, 128:256] = vi - vr
            ref[j, :, 256:384] = vr + vi
        else:
            ref[j, :, 0:128] = vr + vi
            ref[j, :, 128:256] = vr
            ref[j, :, 256:384] = vi

    def b_dft(s):
        s = jnp.minimum(s, NSL - 1)
        d0 = pl.multiple_of(s * SL, SL)
        HP = SL // 2
        prev = None
        sgn = jnp.where(lax.broadcasted_iota(jnp.int32, (SL, 128), 1) < 64, 1.0, -1.0)
        for jb in range(4):
            yield "m", 120
            lhs = jnp.concatenate([uin_ref[pl.ds(d0, SL), 128 * j:128 * (j + 1)] for j in range(4 * jb, 4 * jb + 4)], axis=0)
            o = jnp.dot(lhs, FT_ref[...], preferred_element_type=f32)
            for k in range(4):
                j = 4 * jb + k
                ur, ui = o[k * SL:(k + 1) * SL, 0:128], o[k * SL:(k + 1) * SL, 128:256]
                if prev is None:
                    put_bu(ut_ref, j, ur, ui, False)
                else:
                    put_bu(ut_ref, j, ur - sgn * prev[1], ui + sgn * prev[0], False)
                prev = (ur, ui)
        tiles = {}
        for up in range(2):
            yield "v", 150
            for blk in range(4):
                parts = [kt_ref[up, pl.ds(ch * 4 + blk, HP, stride=8), :] for ch in range(2)]
                tiles[(up, blk)] = jnp.concatenate(parts, axis=0).astype(bf16)
        by_g = {}
        for (m, up, blk, gi) in _PLAN:
            by_g.setdefault(gi, []).append((m, up, blk))
        res = {}
        dcol = col_ref[1, pl.ds(d0, SL), :]
        for gi in range(6):
            yield "m", 120
            lst = by_g[gi]
            lhs = jnp.concatenate([tiles[(up, blk)] for (_, up, blk) in lst], axis=0)
            o = jnp.dot(lhs, GT_ref[gi], preferred_element_type=f32)
            for k, (m, _, _) in enumerate(lst):
                piece = o[k * SL:(k + 1) * SL]
                res[m] = piece if m not in res else res[m] + piece
            for m in sorted(set(x_[0] for x_ in lst)):
                if gi == 1:
                    continue
                vr, vi = res[m][:, 0:128], res[m][:, 128:256]
                if m == 0:
                    vr = vr + dcol
                put_bu(bm_ref, m, vr, vi, True)

    def b_conv(i_lo, i_hi):
        for i in range(i_lo, i_hi):
            for v in range(SL // 8):
                rs = slice(8 * v, 8 * (v + 1))
                a1 = a2 = a3 = None
                for m in range(i + 1):
                    if m % 2 == 0:
                        yield "v", 8 * min(2, i + 1 - m)
                    j = i - m
                    if G3:
                        p1 = bm_ref[m, rs, 0:128] * ut_ref[j, rs, 0:128]
                        p2 = bm_ref[m, rs, 128:256] * ut_ref[j, rs, 128:256]
                        p3 = bm_ref[m, rs, 256:384] * ut_ref[j, rs, 256:384]
                        a3 = p3 if a3 is None else a3 + p3
                    else:
                        p1, p2 = cmul(bm_ref[m, rs, 0:128], bm_ref[m, rs, 128:256], ut_ref[j, rs, 0:128], ut_ref[j, rs, 128:256])
                    a1 = p1 if a1 is None else a1 + p1
                    a2 = p2 if a2 is None else a2 + p2
                if G3:
                    yr, yi = a1 - a3, a1 + a2
                else:
                    yr, yi = a1, a2
                yh_ref[i * SL + 8 * v:i * SL + 8 * (v + 1), 0:128] = yr
                yh_ref[i * SL + 8 * v:i * SL + 8 * (v + 1), 128:256] = yi
    conv_cost = lambda a, b: sum(32 * (i + 1) for i in range(a, b))

    MAXMM = int(E("MAXMM", "1"))
    MM1, MM2 = E("MM", "10")[0] == "1", E("MM", "10")[1] == "1"
    def b_step(k, s):
        if LAY == "a":
            if k == 0:
                return chain(b_inv(s - 1), b_tables(s, 0, 4)), 4 * T_OCT + 400
            if k == 1:
                return b_kgen(s, 0, 16), 16 * G_PAIR
            if k == 2:
                return b_dft(s), 1500
            return b_conv(0, 16), conv_cost(0, 16)
        if LAY == "c":
            GS, CS = int(E("GS", "8")), int(E("CS", "12"))
            if k == 0:
                return chain(b_conv(CS, 16), b_kgen(s, 0, GS)), conv_cost(CS, 16) + GS * G_PAIR
            if k == 1:
                return chain(b_kgen(s, GS, 16)), (16 - GS) * G_PAIR
            if k == 2:
                return chain(b_inv(s - 1), b_dft(s)), 1900
            return b_conv(0, CS), conv_cost(0, CS)
        if LAY == "b":
            CS = 12
            if k == 0:
                return chain(b_conv(CS, 16), b_kgen(s, 0, 8)), conv_cost(CS, 16) + 8 * G_PAIR
            if k == 1:
                return chain(b_inv(s - 1), b_kgen(s, 8, 16)), 400 + 8 * G_PAIR
            if k == 2:
                return chain(b_dft(s), b_tables(s + 1, 0, 2)), 1500 + 2 * T_OCT
            return chain(b_tables(s + 1, 2, 4), b_conv(0, CS)), conv_cost(0, CS) + 2 * T_OCT

    def stage(i, s_new, m_new, s_old, m_old, do_q=True, do_e=True, bwork=None, speed=1.0, pump=None, span=(0.0, 1.0), mmf=None):
        nchunk = S // R
        own = pump is None
        if own:
            pump = Pump(*bwork) if bwork is not None else Pump(None, 0)
        prog = lambda x: speed * (span[0] + (span[1] - span[0]) * x)
        m1, m2, mx = mmf if mmf is not None else (MM1, MM2, MAXMM)
        if do_e:
            h = i % 16
            q0 = pl.multiple_of((i // 16) * NQ, NQ)
            r0 = pl.multiple_of(h * 16, 16)
            mo = jnp.max(m_old[...], axis=0, keepdims=True)
        if do_q:
            hq = (i + 1) % 16
            qq0 = pl.multiple_of((((i + 1) // 16) % 4) * NQ, NQ)
            h4 = hq // 4
            qm = upk(qm_ref[hq, :, pl.ds(qq0, NQ)])
        mrun = None
        acc = None
        LASTEQ = int(E("LASTEQ", "1"))
        for c in range(nchunk):
            rs = slice(c * R, (c + 1) * R)
            eq = do_q and do_e and c >= nchunk - LASTEQ and span[1] == 1.0
            if do_q and not eq:
                s = jnp.dot(upk(k_ref[h4, c * R // 2:(c + 1) * R // 2, :]), qm, preferred_element_type=f32)
            if do_e:
                p = jnp.exp2(s_old[rs, :] - mo).astype(bf16)
            if eq:
                d_ = jnp.dot(upk(vt_ref[pl.ds(r0, 16), rs]), p, preferred_element_type=f32)
                acc = d_ if acc is None else acc + d_
                s = jnp.dot(upk(k_ref[h4, c * R // 2:(c + 1) * R // 2, :]), qm, preferred_element_type=f32)
            pump.to(prog((2 * c + 1) / (2 * nchunk)), mm=m1, max_mm=mx)
            if do_q:
                s_new[rs, :] = s
                mc = jnp.max(s.reshape(R // 8, 8, NQ), axis=0)
                mrun = mc if mrun is None else jnp.maximum(mrun, mc)
            if do_e and not eq:
                d_ = jnp.dot(upk(vt_ref[pl.ds(r0, 16), rs]), p, preferred_element_type=f32)
                acc = d_ if acc is None else acc + d_
            pump.to(prog((2 * c + 2) / (2 * nchunk)), mm=m2, max_mm=mx)
        if own or span[1] == 1.0:
            pump.finish()
        if do_q:
            m_new[...] = mrun
        if do_e:
            o = acc / acc[28:29, :]
            ot_ref[pl.ds(pl.multiple_of(h * 32, 32), 32), pl.ds(q0, NQ)] = o.astype(bf16)

    def out_proj(qb):
        q0 = pl.multiple_of(qb * NQ, NQ)
        oa = lax.dot_general(ot_ref[:, pl.ds(q0, NQ)], upk(wop_ref[...]), TN, preferred_element_type=f32)
        ost_ref[pl.ds(q0, NQ), 0:448] = oa.astype(bf16)

    def out_proj_items(qb):
        q0 = pl.multiple_of(qb * NQ, NQ)
        w_ = upk(wop_ref[...])
        for rb in range(NQ // 128):
            yield "m", 1
            cs = pl.ds(q0 + 128 * rb, 128)
            oa = lax.dot_general(ot_ref[:, cs], w_, TN, preferred_element_type=f32)
            ost_ref[cs, 0:448] = oa.astype(bf16)

    QL = S - NQ
    def out_proj_partial():
        for rb in range(NQ // 128):
            yield "m", 1
            cs = slice(QL + 128 * rb, QL + 128 * (rb + 1))
            opart_ref[128 * rb:128 * (rb + 1), :] = lax.dot_general(ot_ref[0:384, cs], upk(wop_ref[0:192, :]), TN, preferred_element_type=f32)

    def finish_b():
        for tb in range(S // 128):
            yield "v", 1
            rs = slice(128 * tb, 128 * (tb + 1))
            yb = yt_ref[:, rs].T
            ost_ref[rs, 448:896] = yb[:, 64:512]

    def out_copy(qb):
        return pltpu.make_async_copy(ost_ref.at[pl.ds(qb * NQ, NQ)], out_hbm.at[pl.ds(qb * NQ, NQ)], sem_out.at[qb])
    NLC = int(E("NLC", "4"))
    LC = NQ // NLC
    def last_copy(c):
        return pltpu.make_async_copy(ost_ref.at[pl.ds(QL + c * LC, LC), pl.ds(0, 512)], out_hbm.at[pl.ds(QL + c * LC, LC), pl.ds(0, 512)], sem_out.at[4 + c])
    def lastb_copy():
        return pltpu.make_async_copy(ost_ref.at[pl.ds(QL, NQ), pl.ds(512, 384)], out_hbm.at[pl.ds(QL, NQ), pl.ds(512, 384)], sem_out.at[3])

    n_units = 16 * (S // NQ)
    sep = (lambda f: pl.when(zz == 0)(f)) if CFG["sep"] else (lambda f: f())
    def b_unit(i, k, s):
        bufs = (sB, mB, sA, mA) if k % 2 == 0 else (sA, mA, sB, mB)
        with SC(f'stageB{k}'):
            stage(i, *bufs, bwork=b_step(k, s), speed=float(E('SP%d' % k, '1.0')))

    if LAY == "d":
        bm_ref[...] = jnp.zeros(bm_ref.shape, f32)
        ut_ref[...] = jnp.zeros(ut_ref.shape, f32)
    stage(-1, sA, mA, None, None, do_e=False)
    with SC('wait_last'):
        for cp in cp_c + [cp_u]:
            cp.wait()

    def body_s(i, c):
        s = i // 4
        for k in range(4):
            @pl.when(i % 4 == k)
            def _():
                b_unit(i, k, s)
        @pl.when(i % 16 == 15)
        def _():
            with SC('outproj'):
                out_proj(i // 16)
        return c
    def body_m(s, c):
        for k in range(4):
            b_unit(4 * s + k, k, s)
        @pl.when(s % 4 == 3)
        def _():
            with SC('outproj'):
                out_proj(s // 4)
        return c
    def body2(j, c):
        i = first2 + 2 * j
        bufs = ((sB, mB, sA, mA), (sA, mA, sB, mB))
        sep(lambda: stage(i, *bufs[first2 % 2]))
        sep(lambda: stage(i + 1, *bufs[(first2 + 1) % 2]))
        return c
    def pair(i, gen, total, sp, mmf=None):
        pmp = Pump(gen, total)
        stage(i, sB, mB, sA, mA, pump=pmp, span=(0.0, 0.5), speed=sp, mmf=mmf)
        stage(i + 1, sA, mA, sB, mB, pump=pmp, span=(0.5, 1.0), speed=sp, mmf=mmf)
    mmf_of = lambda k, d: (E(k, d)[0] == "1", E(k, d)[1] == "1", int(E(k, d)[2]))
    with SC('loop'):
        if LAY == "d":
            mk = lambda f: (lambda *its: mix(*its)) if f else (lambda *its: chain(*[g for g, _ in its]))
            combA, combB = mk(E("MIXA", "1") == "1"), mk(E("MIXB", "0") == "1")
            OPIN = E("OPIN", "1") == "1"
            def blkA(s, op=False):
                d_ = dict(G=(b_kgen(s, 0, 16), 16 * G_PAIR), C=(b_conv(0, 16), conv_cost(0, 16)))
                its = [d_[k] for k in E("ORDA", "GC")]
                if op:
                    def scaled(gen, f):
                        for kind, cost in gen:
                            yield kind, cost * f
                    its.append((scaled(out_proj_items(s // 4 - 1), int(E("OPS", "1000"))), 4 * int(E("OPS", "1000"))))
                pair(4 * s, combA(*its), sum(t for _, t in its), float(E("SPA0" if op else "SPA", "1.15")), mmf_of("MA0" if op else "MA", "102"))
            def blkB(s):
                d_ = dict(F=(b_dft(s), int(E("CF", "1500"))), I=(b_inv(s - 1), int(E("CI", "400"))), T=(b_tables(s + 1, 0, 4), 4 * T_OCT))
                its = [d_[k] for k in E("ORDB", "FIT")]
                pair(4 * s + 2, combB(*its), sum(t for _, t in its), float(E("SPB", "1.15")), mmf_of("MB", "111"))
                if not OPIN:
                    @pl.when(s % 4 == 3)
                    def _():
                        out_proj(s // 4)
            def body_d(j, c):
                s = j // 2
                if OPIN:
                    ev = lambda: lax.cond((s % 4 == 0) & (s > 0), lambda: blkA(s, True), lambda: blkA(s))
                else:
                    ev = lambda: blkA(s)
                lax.cond(j % 2 == 0, ev, lambda: blkB(s))
                return c
            if E("BRD", "1") == "1":
                lax.fori_loop(0, 2 * NSL, body_d, 0)
            else:
                def body_dm(s, c):
                    blkA(s)
                    blkB(s)
                    return c
                lax.fori_loop(0, NSL, body_dm, 0)
        elif E('BR', '1') == '1':
            lax.fori_loop(0, 4 * NSL, body_s, 0)
        elif E('BR', '1') == '3':
            def body_c(i, c):
                s = i // 4
                def k3():
                    b_unit(i, 3, s)
                    @pl.when(s % 4 == 3)
                    def _():
                        out_proj(s // 4)
                lax.cond(i % 4 < 2,
                         lambda: lax.cond(i % 2 == 0, lambda: b_unit(i, 0, s), lambda: b_unit(i, 1, s)),
                         lambda: lax.cond(i % 2 == 0, lambda: b_unit(i, 2, s), k3))
                return c
            lax.fori_loop(0, 4 * NSL, body_c, 0)
        else:
            lax.fori_loop(0, NSL, body_m, 0)
        i0 = 4 * NSL
        bufs = lambda i: (sB, mB, sA, mA) if i % 2 == 0 else (sA, mA, sB, mB)
        def once(f):
            if E("ONCE", "1") == "1":
                lax.fori_loop(0, 1 + zz, lambda _, c: (f(), c)[1], 0)
            else:
                pl.when(zz == 0)(f)
        once(lambda: pair(i0, chain(b_conv(0, 16)), conv_cost(0, 16), float(E("SPC", "2.0"))) if E("PP", "0") == "1" else
             stage(i0, *bufs(i0), bwork=(b_conv(0, 16), conv_cost(0, 16)), speed=float(E("SPC", "1.1"))))
        once(lambda: stage(i0 + 1, *bufs(i0 + 1), bwork=(b_inv(NSL - 1), 400), speed=float(E("SPI", "1.5"))))
        once(lambda: stage(i0 + 2, *bufs(i0 + 2), bwork=(finish_b(), S // 128), speed=float(E("SPF", "1.3"))))
        first2 = i0 + 3
        for qb in range(3):
            out_copy(qb).start()
        lastb_copy().start()
        n2 = (n_units - 1 - first2) // 2
        lax.fori_loop(0, n2, body2, 0)
        for i in range(first2 + 2 * n2, n_units - 1):
            stage(i, *bufs(i))
        stage(n_units - 1, None, None, sB, mB, do_q=False, bwork=(out_proj_partial(), NQ // 128), speed=1.5)
    with SC('tail'):
        wlast = upk(wop_ref[192:256, :])
        for c in range(NLC):
            for rb in range(c * LC // 128, (c + 1) * LC // 128):
                cs = slice(QL + 128 * rb, QL + 128 * (rb + 1))
                oa = opart_ref[128 * rb:128 * (rb + 1), :] + lax.dot_general(ot_ref[384:512, cs], wlast, TN, preferred_element_type=f32)
                ost_ref[cs, 0:448] = oa.astype(bf16)
            last_copy(c).start()
        for qb in range(3):
            out_copy(qb).wait()
        lastb_copy().wait()
        for c in range(NLC):
            last_copy(c).wait()


@jax.jit
def pallas_concat_heads__mha_block__ssm_conv_s4__prompt_kernel(A_x, A_wqkv, A_wo, B_u, B_A_re, B_A_im, B_B_re, B_B_im, B_C_re, B_C_im, B_log_dt, B_Dskip):
    V = pltpu.VMEM
    FW = 384 if CFG["g3"] else 256
    TD = D if E("TPRO", "0") == "1" else SL
    scratch = [
        V((D,), bf16), V((D,), bf16), V((D, S), bf16), V((D, 3 * D), bf16), V((D, D), bf16), V((D, S), bf16), V((6, D, N), bf16),
        V((128, 256), bf16), V((256, 128), bf16), V((6, 128, 256), bf16), V((S, 2 * D), bf16),
        V((704, 512), i32), V((3, 256, 512), i32), V((256, D), i32),
        V((16, 64, S), i32), V((4, S // 2, 128), i32), V((256, S), i32),
        V((S, NQ), f32), V((S, NQ), f32), V((8, NQ), f32), V((8, NQ), f32), V((512, S), bf16),
        V((2, D, 128), f32),
        V((4, 8 * TD, 128), i32), V((4, 8 * TD, 128), f32), V((4, TD, 128), f32),
        V((2, 8 * (SL // 2), 128), f32),
        V((16, SL, FW), f32), V((16, SL, FW), f32),
        V((512, S), bf16), V((16 * SL, 256), f32), V((NQ, D), f32),
        pltpu.SemaphoreType.DMA((20,)), pltpu.SemaphoreType.DMA((12,)),
    ]
    anyspec = pl.BlockSpec(memory_space=pl.ANY)
    vspec = pl.BlockSpec(memory_space=pltpu.VMEM)
    out = pl.pallas_call(
        kernel,
        out_shape=jax.ShapeDtypeStruct((S, 2 * D), bf16),
        in_specs=[pl.BlockSpec(memory_space=pltpu.SMEM)] + [anyspec] * 15,
        out_specs=anyspec,
        scratch_shapes=scratch,
        compiler_params=pltpu.CompilerParams(vmem_limit_bytes=124 * 1024 * 1024, flags=FLAGS or None),
    )(np.zeros((1,), np.int32), A_x.reshape(S, D).T, A_wqkv, A_wo, B_u.reshape(S, D).T, B_A_re, B_A_im, B_B_re, B_B_im, B_C_re, B_C_im, B_log_dt, B_Dskip,
      C_FT, C_FINVT, C_GT)
    return out.reshape(1, S, 2 * D)
```

```python
import functools, contextlib
import numpy as np
import jax
import jax.numpy as jnp
from jax import lax
import jax.experimental.pallas as pl
import jax.experimental.pallas.tpu as pltpu
import ml_dtypes

S, D, H, DH, N = 2048, 448, 16, 28, 256
NQ = 512
R = 128
SL = 32
NSL = D // SL
NCB = 4
CB = S // NCB
NT = (((1,), (1,)), ((), ()))
TN = (((0,), (0,)), ((), ()))
f32, bf16, i32 = jnp.float32, jnp.bfloat16, jnp.int32
LOG2E = 1.4426950408889634

def _rbf16(l):
    x = np.asarray(l, np.float32)
    u = x.view(np.uint32).astype(np.uint64)
    u = (u + 0x7FFF + ((u >> 16) & 1)) & 0xFFFF0000
    return u.astype(np.uint32).view(np.float32).astype(np.float64)

HI = np.array([0, 1, 2, 3, 4, 5, 6, 7, 512, 516, 1024, 1536, 640, 1152, 1664, 0])

def dft_consts():
    T, M = 128, 256
    forder = np.concatenate([np.arange(0, 128, 2), np.arange(1, 128, 2)])
    ang = 2 * np.pi * (forder[:, None] + 0.5) * np.arange(T)[None, :] / M
    F = np.concatenate([np.cos(ang), -np.sin(ang)], 0)
    Finv = np.concatenate([np.cos(ang).T, -np.sin(ang).T], 1) * (2.0 / M)
    def lag_of(upper, blk):
        r = np.arange(8)[:, None] + (8 if upper else 0)
        b = 16 * blk + np.arange(16)[None, :]
        return (HI[r] + 8 * b).reshape(-1)
    plan = []
    Gs = []
    for m in range(16):
        tgt = _rbf16(128 * m + np.arange(T)).astype(int)
        if m < 4: cand = [(0, m)] + ([(0, m + 1)] if m == 2 else []) + ([(1, 0)] if m == 3 else [])
        elif m < 8: cand = [(1, m - 4)]
        elif m < 12: cand = [(1, m - 8)]
        else: cand = [(1, m - 12)]
        used = np.zeros(T, bool)
        for (up, blk) in cand:
            lg = lag_of(up, blk)
            valid = np.ones(128, bool)
            if up: valid[7 * 16:] = False
            E = np.zeros((T, 128))
            for j in range(T):
                if used[j]: continue
                idx = np.where((lg == tgt[j]) & valid)[0]
                if len(idx):
                    E[j, idx[0]] = 1; used[j] = True
            Gm = F @ E
            gi = None
            for k, g0 in enumerate(Gs):
                if np.array_equal(g0, Gm): gi = k
            if gi is None:
                Gs.append(Gm); gi = len(Gs) - 1
            plan.append((m, up, blk, gi))
        assert used.all()
    return F, Finv, np.stack(Gs), plan


_F, _FINV, _G, _PLAN = dft_consts()
_bf = lambda a: np.asarray(a, np.float32).astype(ml_dtypes.bfloat16)
C_FT = _bf(_F.T)
C_FINVT = _bf(_FINV.T)
C_GT = _bf(np.transpose(_G, (0, 2, 1)))
FLAGS = {}
_KNOBS = {'TPRO': '0', 'LAYOUT': 'd', 'ONCE': '1', 'MIXA': '1', 'GSPL': '1', 'G3': '1', 'MIXB': '0', 'LASTEQ': '1', 'OPS': '100', 'SPA0': '1.2', 'SPA': '1.25', 'PORD': '1', 'OPIN': '1', 'N2': '2', 'PLOOP': '0', 'MB': '111', 'ORDB': 'TIF', 'SPB': '0.97', 'CF': '1500', 'ORDA': 'CG', 'OPT': '1'}
E = _KNOBS.get
CFG = dict(g3=E("G3", "1") == "1", layout=E("LAYOUT", "a"), sep=E("SEP", "0") == "1")
pk = lambda x: pltpu.bitcast(x, i32)
upk = lambda x: pltpu.bitcast(x, bf16)


def cmul(ar, ai, br, bi):
    return ar * br - ai * bi, ar * bi + ai * br


def sincos(x):
    k = jnp.round(x * 0.6366197723675814)
    r = x - k * 1.5703125
    r = r - k * 4.837512969970703125e-4
    r = r - k * 7.54978995489188e-8
    r2 = r * r
    s = r + r * r2 * (-1.6666654611e-1 + r2 * (8.3321608736e-3 + r2 * -1.9515295891e-4))
    c = 1.0 + r2 * (-0.5 + r2 * (4.166664568298827e-2 + r2 * (-1.388731625493765e-3 + r2 * 2.443315711809948e-5)))
    q = k.astype(jnp.int32)
    swap = (q & 1) != 0
    s1 = jnp.where(swap, c, s)
    c1 = jnp.where(swap, s, c)
    s1 = jnp.where((q & 2) != 0, -s1, s1)
    c1 = jnp.where(((q + 1) & 2) != 0, -c1, c1)
    return s1, c1


def fold8(t):
    sub = lax.broadcasted_iota(jnp.int32, (8, 128), 0)
    seg = lax.broadcasted_iota(jnp.int32, (8, 128), 1) >> 4
    for k in (4, 2, 1):
        sb = (sub & k) != 0
        gb = (seg & k) != 0
        up = pltpu.roll(pltpu.roll(t, 8 - k, 0), 16 * k, 1)
        dn = pltpu.roll(pltpu.roll(t, k, 0), 128 - 16 * k, 1)
        t = jnp.where(sb == gb, t, jnp.where(gb, up, dn))
    return t


def sub_transpose8(xs):
    xs = list(xs)
    sub = lax.broadcasted_iota(jnp.int32, (8, 128), 0)
    for k in (4, 2, 1):
        keep = (sub & k) == 0
        new = list(xs)
        for a in range(8):
            if a & k:
                continue
            b = a ^ k
            new[a] = jnp.where(keep, xs[a], pltpu.roll(xs[b], k, 0))
            new[b] = jnp.where(keep, pltpu.roll(xs[a], 8 - k, 0), xs[b])
        xs = new
    return xs


def sel_matrix(rows0, nrows, col0, ncols, off):
    p = rows0 + lax.broadcasted_iota(jnp.int32, (nrows, ncols), 0)
    c = col0 + lax.broadcasted_iota(jnp.int32, (nrows, ncols), 1)
    j = p & 31
    src = off + 28 * (p >> 5) + j
    return jnp.where((src == c) & (j < 28), 1.0, 0.0).astype(bf16)


class Pump:
    def __init__(self, gen, total):
        self.gen, self.total, self.done = gen, total, 0.0
        self.pending = next(gen, None) if gen is not None else None
    def to(self, frac, mm=True, max_mm=99):
        n_mm = 0
        while self.pending is not None and self.done < frac * self.total - 1e-9:
            kind, cost = self.pending
            if kind == "m":
                if not mm or n_mm >= max_mm:
                    break
                n_mm += 1
            self.done += cost
            self.pending = next(self.gen, None)
    def finish(self):
        while self.pending is not None:
            self.pending = next(self.gen, None)


def chain(*gens):
    for g_ in gens:
        yield from g_


def mix(*items):
    st = [[g, float(t), 0.0, next(g, None)] for g, t in items]
    while True:
        live = [x for x in st if x[3] is not None]
        if not live:
            return
        x = min(live, key=lambda y: y[2] / y[1])
        kind, cost = x[3]
        yield kind, cost
        x[2] += cost
        x[3] = next(x[0], None)


def kernel(z_ref, xt_hbm, wqkv_hbm, wo_hbm, ut_hbm, are_hbm, aim_hbm, bre_hbm, bim_hbm, cre_hbm, cim_hbm, ldt_hbm, dsk_hbm,
           FT_hbm, FinvT_hbm, GT_hbm,
           out_hbm,
           ldt_ref, dsk_ref, xt_ref, wqkv_ref, wo_ref, uin_ref, par_ref, FT_ref, FinvT_ref, GT_ref, ost_ref,
           wt_ref, wp_ref, wop_ref, qm_ref, k_ref, vt_ref, sA, sB, mA, mB, ot_ref,
           col_ref, a_tab, v0_tab, y8_tab, kt_ref, bm_ref, ut_ref, yt_ref, yh_ref, opart_ref, opt_ref, wopt_ref, sem_in, sem_out):
    SC = (lambda n: jax.named_scope(n)) if False else (lambda n: contextlib.nullcontext())
    zz = z_ref[0]
    OPT = E('OPT', '1') == '1'
    LAY = CFG["layout"]
    GSPL = E("GSPL", "1") == "1"
    TPRO = E("TPRO", "0") == "1"
    par_hbm = (are_hbm, aim_hbm, bre_hbm, bim_hbm, cre_hbm, cim_hbm)
    WOFF = ((384, 512), (896, 448), (0, 512))
    cp_w = [pltpu.make_async_copy(wqkv_hbm.at[:, pl.ds(a, n)], wqkv_ref.at[:, pl.ds(a, n)], sem_in.at[k])
            for k, (a, n) in enumerate(((384, 512), (896, 448), (0, 384)))]
    cp_x = [pltpu.make_async_copy(xt_hbm.at[:, pl.ds(cb * CB, CB)], xt_ref.at[:, pl.ds(cb * CB, CB)], sem_in.at[3 + cb]) for cb in range(NCB)]
    cp_p = [pltpu.make_async_copy(par_hbm[k], par_ref.at[k], sem_in.at[7 + k]) for k in range(6)]
    cp_wo = pltpu.make_async_copy(wo_hbm, wo_ref, sem_in.at[13])
    cp_c = [pltpu.make_async_copy(a, b, sem_in.at[14 + k]) for k, (a, b) in
            enumerate(((FT_hbm, FT_ref), (FinvT_hbm, FinvT_ref), (GT_hbm, GT_ref)))]
    cp_u = pltpu.make_async_copy(ut_hbm, uin_ref, sem_in.at[17])
    cp_v = [pltpu.make_async_copy(ldt_hbm, ldt_ref, sem_in.at[18]), pltpu.make_async_copy(dsk_hbm, dsk_ref, sem_in.at[19])]
    for cp in ([cp_w[0], cp_x[0], cp_w[1], cp_w[2], cp_x[1]] if E('PORD', '0') == '0' else [cp_w[0], cp_x[0], cp_w[1], cp_x[1], cp_w[2]]) + cp_x[2:] + [cp_wo] + cp_v + cp_p + cp_c + [cp_u]:
        cp.start()

    yt_ref[0:64, :] = jnp.zeros((64, S), bf16)
    yh_ref[...] = jnp.zeros(yh_ref.shape, f32)
    def w_transpose(tiles):
        for c in tiles:
            c1 = min(128 * (c + 1), 3 * D)
            blk = wqkv_ref[:, 128 * c:c1]
            blk = jnp.concatenate([blk, jnp.zeros((512 - D, c1 - 128 * c), bf16)], axis=0)
            if c1 - 128 * c < 128:
                blk = jnp.concatenate([blk, jnp.zeros((512, 128 - (c1 - 128 * c)), bf16)], axis=1)
            wt_ref[64 * c:64 * (c + 1), :] = pk(blk.T)
    def w_respace(part, hs=range(16)):
        z2 = jnp.zeros((2, 512), i32)
        for h in hs:
            r0 = (D * part + DH * h) // 2
            wp_ref[part, 16 * h:16 * (h + 1), :] = jnp.concatenate([wt_ref[r0:r0 + 14, :], z2], axis=0)
    def w_prep_vq():
        for c in (7, 8, 9, 10, 0, 1, 2):
            yield "v", 2
            w_transpose((c,))
        for part in (2, 0):
            for h in range(0, 16, 4):
                yield "v", 1
                w_respace(part, range(h, h + 4))

    def b_tables(s, v_lo, v_hi, voff=None):
        s = min(s, NSL - 1) if isinstance(s, int) else jnp.minimum(s, NSL - 1)
        d0 = s * SL if isinstance(s, int) else pl.multiple_of(s * SL, SL)
        if TPRO:
            trow = lambda v, c_: pl.ds(pl.multiple_of(8 * (d0 + 8 * v + c_), 8), 8)
            yrow = lambda v: pl.ds(pl.multiple_of(d0 + 8 * v, 8), 8)
        elif voff is None:
            trow = lambda v, c_: slice((8 * v + c_) * 8, (8 * v + c_) * 8 + 8)
            yrow = lambda v: slice(8 * v, 8 * v + 8)
        else:
            trow = lambda v, c_: pl.ds(pl.multiple_of(64 * (voff + v) + 8 * c_, 8), 8)
            yrow = lambda v: pl.ds(pl.multiple_of(8 * (voff + v), 8), 8)
        for v in range(v_lo, v_hi):
            rs = pl.ds(pl.multiple_of(d0 + 8 * (v if voff is None else voff + v), 8), 8)
            dt = col_ref[0, rs, :]
            for t in range(2):
                ls = slice(128 * t, 128 * (t + 1))
                ld = lambda k: par_ref[k, rs, ls].astype(f32)
                yield "v", 100
                a_re, a_im = dt * ld(0), dt * ld(1)
                mag = jnp.exp(a_re)
                if E("SINCOS", "0") == "1":
                    sn, cs = sincos(a_im)
                    zr = mag * cs
                    z = (zr, mag * sn)
                else:
                    zr = mag * jnp.cos(a_im)
                    yield "v", 60
                    z = (zr, mag * jnp.sin(a_im))
                yield "v", 60
                z2 = cmul(*z, *z)
                z4 = cmul(*z2, *z2)
                y = cmul(*z4, *z4)
                rows_ = [(jnp.ones_like(zr), jnp.zeros_like(zr)), y]
                for r in range(6):
                    rows_.append(cmul(*rows_[-1], *y))
                yield "v", 70
                tr = sub_transpose8([x_[0] for x_ in rows_])
                for c_ in range(8):
                    v0_tab[t, trow(v, c_), :] = tr[c_]
                yield "v", 70
                ti = sub_transpose8([x_[1] for x_ in rows_])
                for c_ in range(8):
                    v0_tab[2 + t, trow(v, c_), :] = ti[c_]
                yield "v", 40
                z16 = cmul(*y, *y)
                z32 = cmul(*z16, *z16)
                z64 = cmul(*z32, *z32)
                y8_tab[t, yrow(v), :] = z64[0]
                y8_tab[2 + t, yrow(v), :] = z64[1]
                z128 = cmul(*z64, *z64)
                z256 = cmul(*z128, *z128)
                z512 = cmul(*z256, *z256)
                pe = lambda a, b: pltpu.pack_elementwise([a, b], packed_dtype=bf16)
                wr_, wi_ = [], []
                def put_pair(x0, x1):
                    wr_.append(pe(x0[0], x1[0]))
                    wi_.append(pe(-x0[1], -x1[1]))
                yield "v", 40
                w = cmul(ld(4), ld(5), dt * ld(2), dt * ld(3))
                cur = w
                for j in range(4):
                    nxt = cmul(*cur, *z)
                    put_pair(cur, nxt)
                    if j < 3:
                        cur = cmul(*nxt, *z)
                    if j == 1:
                        yield "v", 30
                yield "v", 50
                w512 = cmul(*w, *z512)
                put_pair(w512, cmul(*w512, *z4))
                w1024 = cmul(*w512, *z512)
                w1536 = cmul(*w1024, *z512)
                put_pair(w1024, w1536)
                put_pair(cmul(*w512, *z128), cmul(*w1024, *z128))
                zero = jnp.zeros_like(zr)
                put_pair(cmul(*w1536, *z128), (zero, zero))
                yield "v", 75
                wr = sub_transpose8(wr_)
                for c_ in range(8):
                    a_tab[t, trow(v, c_), :] = wr[c_]
                yield "v", 75
                wi = sub_transpose8(wi_)
                for c_ in range(8):
                    a_tab[2 + t, trow(v, c_), :] = wi[c_]
    T_OCT = 2 * (620 if E("SINCOS", "0") == "1" else 680)

    scale = (DH ** -0.5) * LOG2E
    tpump = [None]
    tcount, tden = [0], [36]
    def proj(part, cb, gs=range(4)):
        if isinstance(cb, int):
            c0 = cb * CB
            cs, cs2 = slice(c0, c0 + CB), slice(c0 // 2, (c0 + CB) // 2)
        else:
            c0 = pl.multiple_of(cb * CB, CB)
            cs, cs2 = pl.ds(c0, CB), pl.ds(pl.multiple_of(cb * (CB // 2), CB // 2), CB // 2)
        xt = xt_ref[:, cs]
        rows = lax.broadcasted_iota(jnp.int32, (128, CB), 0)
        for g in gs:
            o_ = jnp.dot(upk(wp_ref[part, 64 * g:64 * (g + 1), :])[:, 0:D], xt, preferred_element_type=f32)
            if part == 1:
                k_ref[g, cs2, :] = pk(o_.astype(bf16).T)
            elif part == 2:
                vt_ref[64 * g:64 * (g + 1), cs] = pk(jnp.where((rows & 31) == 28, 1.0, o_).astype(bf16))
            else:
                q = o_ * scale
                for hh in range(4):
                    qm_ref[4 * g + hh, :, cs] = pk(jnp.where((rows >> 5) == hh, q, 0.0).astype(bf16))
            if tpump[0] is not None:
                tcount[0] += 1
                tpump[0].to(tcount[0] / tden[0])
    with SC('wait_w'):
        cp_w[0].wait()
    w_transpose((3, 4, 5, 6))
    w_respace(1)
    with SC('wait_x0'):
        cp_x[0].wait()
    if E("PORD", "0") == "0":
        proj(1, 0)
        with SC('wait_wvq'):
            cp_w[1].wait()
            cp_w[2].wait()
            cp_x[1].wait()
        wpump = Pump(w_prep_vq(), 22)
        for g_ in range(4):
            wpump.to((g_ + 1) / 3 * 0.999)
            proj(1, 1, (g_,))
        wpump.finish()
        for part in (2, 0):
            for cb in range(2):
                proj(part, cb)
    else:
        def w_prep(tiles, part):
            for c in tiles:
                yield "v", 2
                w_transpose((c,))
            for h in range(0, 16, 4):
                yield "v", 1
                w_respace(part, range(h, h + 4))
        proj(1, 0, (0, 1, 2))
        with SC('wait_wv'):
            cp_w[1].wait()
        wpump = Pump(w_prep((7, 8, 9, 10), 2), 12)
        wpump.to(0.999)
        proj(1, 0, (3,))
        wpump.finish()
        proj(2, 0)
        with SC('wait_wvq'):
            cp_x[1].wait()
            cp_w[2].wait()
        wpump = Pump(w_prep((0, 1, 2), 0), 10)
        for g_ in range(4):
            wpump.to((g_ + 1) / 3 * 0.999)
            proj(1, 1, (g_,))
        wpump.finish()
        proj(2, 1)
        proj(0, 0)
        proj(0, 1)
    with SC('wait_x23'):
        cp_x[2].wait()
        cp_x[3].wait()
        cp_wo.wait()
        for cp in cp_v + cp_p:
            cp.wait()
    def late_prep():
        yield "v", 6
        ldt = ldt_ref[...].astype(f32).reshape(1, D)
        dsk = dsk_ref[...].astype(f32).reshape(1, D)
        dt_row = jnp.exp(ldt).astype(bf16).astype(f32)
        col_ref[0] = jnp.broadcast_to(dt_row, (128, D)).T
        col_ref[1] = jnp.broadcast_to(dsk, (128, D)).T
        wo = pk(wo_ref[...])
        z2 = jnp.zeros((2, D), i32)
        for h in range(16):
            if h % 4 == 0:
                yield "v", 1
            wop_ref[16 * h:16 * (h + 1), :] = jnp.concatenate([wo[14 * h:14 * h + 14], z2], axis=0)
    def wopt_prep():
        for c in range(4):
            yield "v", 1
            blk = jnp.concatenate([upk(wop_ref[64 * c:64 * (c + 1), :]), jnp.zeros((128, 64), bf16)], axis=1)
            wopt_ref[:, 128 * c:128 * (c + 1)] = pk(blk.T[0:D, :])
    PLOOP = E("PLOOP", "0") == "1"
    lpump = Pump(late_prep(), 10)
    if not PLOOP:
        for g_ in range(4):
            lpump.to((g_ + 1) / 3 * 0.999)
            proj(1, 2, (g_,))
        lpump.finish()
        if LAY in ("b", "d"):
            tden[0] = int(E("TDEN", "17"))
            tpump[0] = Pump(b_tables(0, 0, 4), 4 * T_OCT)
        for part, cb in ((2, 2), (0, 2), (1, 3), (2, 3), (0, 3)):
            proj(part, cb)
        if tpump[0] is not None:
            tpump[0].finish()
    else:
        lpump.finish()
        def pbody(cb, c):
            tcount[0], tden[0] = 0, int(E("TDEN2", "10"))
            tpump[0] = Pump(b_tables(0, 0, 2, voff=2 * (cb - 2)), 2 * T_OCT)
            for part in (1, 2, 0):
                proj(part, cb)
            tpump[0].finish()
            return c
        lax.fori_loop(2, NCB, pbody, 0)

    def b_inv(s):
        r0 = pl.multiple_of(64 + s * SL, SL)
        for ib in range(4):
            yield "m", 100
            lhs = yh_ref[4 * SL * ib:4 * SL * (ib + 1), :].astype(bf16)
            o = jnp.dot(lhs, FinvT_ref[...], preferred_element_type=f32)
            for k in range(4):
                i = 4 * ib + k
                yt_ref[pl.ds(r0, SL), 128 * i:128 * (i + 1)] = o[k * SL:(k + 1) * SL].astype(bf16)

    def b_kgen(s, g_lo, g_hi):
        lane = lax.broadcasted_iota(jnp.int32, (8, 128), 1)
        HP = SL // 2
        if TPRO:
            d0 = pl.multiple_of(jnp.minimum(s, NSL - 1) * SL, SL)
        for g in range(g_lo, g_hi):
            def row(d, n):
                if TPRO:
                    return pl.ds(pl.multiple_of(8 * (d0 + d), 8), 8) if n == 8 else pl.ds(d0 + d, 1)
                return slice(8 * d, 8 * d + 8) if n == 8 else slice(d, d + 1)
            if not GSPL:
                rhs = [[None] * 2 for _ in range(4)]
                lhs = [[None] * 2 for _ in range(4)]
                for ch in range(2):
                    d = g + HP * ch
                    for t in range(2):
                        yield "v", 50
                        vr, vi = v0_tab[t, row(d, 8), :], v0_tab[2 + t, row(d, 8), :]
                        mr = jnp.broadcast_to(y8_tab[t, row(d, 1), :], (8, 128))
                        mi = jnp.broadcast_to(y8_tab[2 + t, row(d, 1), :], (8, 128))
                        rr, ii = [vr], [vi]
                        for j in range(7):
                            nr, ni = cmul(rr[-1], ii[-1], mr, mi)
                            rr.append(nr); ii.append(ni)
                        rhs[t][ch] = jnp.concatenate(rr, axis=0)
                        rhs[2 + t][ch] = jnp.concatenate(ii, axis=0)
                    for t in range(4):
                        lhs[t][ch] = upk(a_tab[t, row(d, 8), :])
                yield "m", 40
                A = jnp.concatenate([jnp.concatenate([lhs[t][0], lhs[t][1]], axis=0) for t in range(4)], axis=1)
                Bm = jnp.concatenate([jnp.concatenate([rhs[t][0], rhs[t][1]], axis=0) for t in range(4)], axis=1).astype(bf16)
                o = lax.dot_general(A, Bm, NT, preferred_element_type=f32)
            else:
                o = None
                for t in range(2):
                    re_, im_ = [], []
                    for ch in range(2):
                        d = g + HP * ch
                        yield "v", 50
                        vr, vi = v0_tab[t, row(d, 8), :], v0_tab[2 + t, row(d, 8), :]
                        mr = jnp.broadcast_to(y8_tab[t, row(d, 1), :], (8, 128))
                        mi = jnp.broadcast_to(y8_tab[2 + t, row(d, 1), :], (8, 128))
                        rr, ii = [vr], [vi]
                        for j in range(7):
                            nr, ni = cmul(rr[-1], ii[-1], mr, mi)
                            rr.append(nr); ii.append(ni)
                        re_.extend(rr)
                        im_.extend(ii)
                    yield "m", 20
                    for kt_, rhs in ((t, re_), (2 + t, im_)):
                        A = jnp.concatenate([upk(a_tab[kt_, row(g + HP * ch, 8), :]) for ch in range(2)], axis=0)
                        d_ = lax.dot_general(A, jnp.concatenate(rhs, axis=0).astype(bf16), NT, preferred_element_type=f32)
                        o = d_ if o is None else o + d_
            yield "v", 40
            t_lo = jnp.where(lane < 64, o[0:8], o[16:24])
            t_hi = jnp.where(lane < 64, o[8:16], o[24:32])
            kt_ref[0, 8 * g:8 * (g + 1), :] = fold8(t_lo)
            kt_ref[1, 8 * g:8 * (g + 1), :] = fold8(t_hi)
    G_PAIR = 280

    G3 = CFG["g3"]
    def put_bu(ref, j, vr, vi, is_b):
        if not G3:
            ref[j, :, 0:128] = vr
            ref[j, :, 128:256] = vi
        elif is_b:
            ref[j, :, 0:128] = vr
            ref[j, :, 128:256] = vi - vr
            ref[j, :, 256:384] = vr + vi
        else:
            ref[j, :, 0:128] = vr + vi
            ref[j, :, 128:256] = vr
            ref[j, :, 256:384] = vi

    def b_dft(s):
        s = jnp.minimum(s, NSL - 1)
        d0 = pl.multiple_of(s * SL, SL)
        HP = SL // 2
        prev = None
        sgn = jnp.where(lax.broadcasted_iota(jnp.int32, (SL, 128), 1) < 64, 1.0, -1.0)
        for jb in range(4):
            yield "m", 120
            lhs = jnp.concatenate([uin_ref[pl.ds(d0, SL), 128 * j:128 * (j + 1)] for j in range(4 * jb, 4 * jb + 4)], axis=0)
            o = jnp.dot(lhs, FT_ref[...], preferred_element_type=f32)
            for k in range(4):
                j = 4 * jb + k
                ur, ui = o[k * SL:(k + 1) * SL, 0:128], o[k * SL:(k + 1) * SL, 128:256]
                if prev is None:
                    put_bu(ut_ref, j, ur, ui, False)
                else:
                    put_bu(ut_ref, j, ur - sgn * prev[1], ui + sgn * prev[0], False)
                prev = (ur, ui)
        tiles = {}
        for up in range(2):
            yield "v", 150
            for blk in range(4):
                parts = [kt_ref[up, pl.ds(ch * 4 + blk, HP, stride=8), :] for ch in range(2)]
                tiles[(up, blk)] = jnp.concatenate(parts, axis=0).astype(bf16)
        by_g = {}
        for (m, up, blk, gi) in _PLAN:
            by_g.setdefault(gi, []).append((m, up, blk))
        res = {}
        dcol = col_ref[1, pl.ds(d0, SL), :]
        for gi in range(6):
            yield "m", 120
            lst = by_g[gi]
            lhs = jnp.concatenate([tiles[(up, blk)] for (_, up, blk) in lst], axis=0)
            o = jnp.dot(lhs, GT_ref[gi], preferred_element_type=f32)
            for k, (m, _, _) in enumerate(lst):
                piece = o[k * SL:(k + 1) * SL]
                res[m] = piece if m not in res else res[m] + piece
            for m in sorted(set(x_[0] for x_ in lst)):
                if gi == 1:
                    continue
                vr, vi = res[m][:, 0:128], res[m][:, 128:256]
                if m == 0:
                    vr = vr + dcol
                put_bu(bm_ref, m, vr, vi, True)

    def b_conv(i_lo, i_hi):
        for i in range(i_lo, i_hi):
            for v in range(SL // 8):
                rs = slice(8 * v, 8 * (v + 1))
                a1 = a2 = a3 = None
                for m in range(i + 1):
                    if m % 2 == 0:
                        yield "v", 8 * min(2, i + 1 - m)
                    j = i - m
                    if G3:
                        p1 = bm_ref[m, rs, 0:128] * ut_ref[j, rs, 0:128]
                        p2 = bm_ref[m, rs, 128:256] * ut_ref[j, rs, 128:256]
                        p3 = bm_ref[m, rs, 256:384] * ut_ref[j, rs, 256:384]
                        a3 = p3 if a3 is None else a3 + p3
                    else:
                        p1, p2 = cmul(bm_ref[m, rs, 0:128], bm_ref[m, rs, 128:256], ut_ref[j, rs, 0:128], ut_ref[j, rs, 128:256])
                    a1 = p1 if a1 is None else a1 + p1
                    a2 = p2 if a2 is None else a2 + p2
                if G3:
                    yr, yi = a1 - a3, a1 + a2
                else:
                    yr, yi = a1, a2
                yh_ref[i * SL + 8 * v:i * SL + 8 * (v + 1), 0:128] = yr
                yh_ref[i * SL + 8 * v:i * SL + 8 * (v + 1), 128:256] = yi
    conv_cost = lambda a, b: sum(32 * (i + 1) for i in range(a, b))

    MAXMM = int(E("MAXMM", "1"))
    MM1, MM2 = E("MM", "10")[0] == "1", E("MM", "10")[1] == "1"
    def b_step(k, s):
        if LAY == "a":
            if k == 0:
                return chain(b_inv(s - 1), b_tables(s, 0, 4)), 4 * T_OCT + 400
            if k == 1:
                return b_kgen(s, 0, 16), 16 * G_PAIR
            if k == 2:
                return b_dft(s), 1500
            return b_conv(0, 16), conv_cost(0, 16)
        if LAY == "c":
            GS, CS = int(E("GS", "8")), int(E("CS", "12"))
            if k == 0:
                return chain(b_conv(CS, 16), b_kgen(s, 0, GS)), conv_cost(CS, 16) + GS * G_PAIR
            if k == 1:
                return chain(b_kgen(s, GS, 16)), (16 - GS) * G_PAIR
            if k == 2:
                return chain(b_inv(s - 1), b_dft(s)), 1900
            return b_conv(0, CS), conv_cost(0, CS)
        if LAY == "b":
            CS = 12
            if k == 0:
                return chain(b_conv(CS, 16), b_kgen(s, 0, 8)), conv_cost(CS, 16) + 8 * G_PAIR
            if k == 1:
                return chain(b_inv(s - 1), b_kgen(s, 8, 16)), 400 + 8 * G_PAIR
            if k == 2:
                return chain(b_dft(s), b_tables(s + 1, 0, 2)), 1500 + 2 * T_OCT
            return chain(b_tables(s + 1, 2, 4), b_conv(0, CS)), conv_cost(0, CS) + 2 * T_OCT

    def stage(i, s_new, m_new, s_old, m_old, do_q=True, do_e=True, bwork=None, speed=1.0, pump=None, span=(0.0, 1.0), mmf=None):
        nchunk = S // R
        own = pump is None
        if own:
            pump = Pump(*bwork) if bwork is not None else Pump(None, 0)
        prog = lambda x: speed * (span[0] + (span[1] - span[0]) * x)
        m1, m2, mx = mmf if mmf is not None else (MM1, MM2, MAXMM)
        if do_e:
            h = i & 15
            q0 = pl.multiple_of((i >> 4) * NQ, NQ)
            r0 = pl.multiple_of(h * 16, 16)
            mo = jnp.max(m_old[...], axis=0, keepdims=True)
        if do_q:
            hq = (i + 1) & 15
            qq0 = pl.multiple_of((((i + 1) >> 4) & 3) * NQ, NQ)
            h4 = hq >> 2
            qm = upk(qm_ref[hq, :, pl.ds(qq0, NQ)])
        mrun = None
        acc = None
        LASTEQ = int(E("LASTEQ", "1"))
        for c in range(nchunk):
            rs = slice(c * R, (c + 1) * R)
            eq = do_q and do_e and c >= nchunk - LASTEQ and span[1] == 1.0
            if do_q and not eq:
                s = jnp.dot(upk(k_ref[h4, c * R // 2:(c + 1) * R // 2, :]), qm, preferred_element_type=f32)
            if do_e:
                p = jnp.exp2(s_old[rs, :] - mo).astype(bf16)
            if eq:
                d_ = jnp.dot(upk(vt_ref[pl.ds(r0, 16), rs]), p, preferred_element_type=f32)
                acc = d_ if acc is None else acc + d_
                s = jnp.dot(upk(k_ref[h4, c * R // 2:(c + 1) * R // 2, :]), qm, preferred_element_type=f32)
            pump.to(prog((2 * c + 1) / (2 * nchunk)), mm=m1, max_mm=mx)
            if do_q:
                s_new[rs, :] = s
                mc = jnp.max(s.reshape(R // 8, 8, NQ), axis=0)
                mrun = mc if mrun is None else jnp.maximum(mrun, mc)
            if do_e and not eq:
                d_ = jnp.dot(upk(vt_ref[pl.ds(r0, 16), rs]), p, preferred_element_type=f32)
                acc = d_ if acc is None else acc + d_
            pump.to(prog((2 * c + 2) / (2 * nchunk)), mm=m2, max_mm=mx)
        if own or span[1] == 1.0:
            pump.finish()
        if do_q:
            m_new[...] = mrun
        if do_e:
            o = acc / acc[28:29, :]
            ot_ref[pl.ds(pl.multiple_of(h * 32, 32), 32), pl.ds(q0, NQ)] = o.astype(bf16)

    def out_proj(qb):
        q0 = pl.multiple_of(qb * NQ, NQ)
        oa = lax.dot_general(ot_ref[:, pl.ds(q0, NQ)], upk(wop_ref[...]), TN, preferred_element_type=f32)
        ost_ref[pl.ds(q0, NQ), 0:448] = oa.astype(bf16)

    def out_proj_items(qb):
        q0 = pl.multiple_of(qb * NQ, NQ)
        w_ = upk(wop_ref[...])
        for rb in range(NQ // 128):
            yield "m", 1
            cs = pl.ds(q0 + 128 * rb, 128)
            if OPT:
                oat = jnp.dot(upk(wopt_ref[...]), ot_ref[:, cs], preferred_element_type=f32)
                oat = jnp.concatenate([oat, jnp.zeros((64, 128), f32)], axis=0).astype(bf16)
                ost_ref[cs, 0:448] = oat.T[:, 0:448]
            else:
                oa = lax.dot_general(ot_ref[:, cs], w_, TN, preferred_element_type=f32)
                ost_ref[cs, 0:448] = oa.astype(bf16)

    QL = S - NQ
    def out_proj_partial():
        for rb in range(NQ // 128):
            yield "m", 1
            cs = slice(QL + 128 * rb, QL + 128 * (rb + 1))
            if OPT:
                opt_ref[:, 128 * rb:128 * (rb + 1)] = jnp.dot(upk(wopt_ref[...])[:, 0:384], ot_ref[0:384, cs], preferred_element_type=f32)
            else:
                opart_ref[128 * rb:128 * (rb + 1), :] = lax.dot_general(ot_ref[0:384, cs], upk(wop_ref[0:192, :]), TN, preferred_element_type=f32)

    def finish_b():
        for tb in range(S // 128):
            yield "v", 1
            rs = slice(128 * tb, 128 * (tb + 1))
            yb = yt_ref[:, rs].T
            ost_ref[rs, 448:896] = yb[:, 64:512]

    def out_copy(qb):
        return pltpu.make_async_copy(ost_ref.at[pl.ds(qb * NQ, NQ)], out_hbm.at[pl.ds(qb * NQ, NQ)], sem_out.at[qb])
    NLC = int(E("NLC", "4"))
    LC = NQ // NLC
    def last_copy(c):
        return pltpu.make_async_copy(ost_ref.at[pl.ds(QL + c * LC, LC), pl.ds(0, 512)], out_hbm.at[pl.ds(QL + c * LC, LC), pl.ds(0, 512)], sem_out.at[4 + c])
    def lastb_copy():
        return pltpu.make_async_copy(ost_ref.at[pl.ds(QL, NQ), pl.ds(512, 384)], out_hbm.at[pl.ds(QL, NQ), pl.ds(512, 384)], sem_out.at[3])

    n_units = 16 * (S // NQ)
    sep = (lambda f: pl.when(zz == 0)(f)) if CFG["sep"] else (lambda f: f())
    def b_unit(i, k, s):
        bufs = (sB, mB, sA, mA) if k % 2 == 0 else (sA, mA, sB, mB)
        with SC(f'stageB{k}'):
            stage(i, *bufs, bwork=b_step(k, s), speed=float(E('SP%d' % k, '1.0')))

    if LAY == "d":
        bm_ref[...] = jnp.zeros(bm_ref.shape, f32)
        ut_ref[...] = jnp.zeros(ut_ref.shape, f32)
    stage(-1, sA, mA, None, None, do_e=False, bwork=(wopt_prep(), 4) if OPT else None, speed=1.4)
    with SC('wait_last'):
        for cp in cp_c + [cp_u]:
            cp.wait()

    def body_s(i, c):
        s = i // 4
        for k in range(4):
            @pl.when(i % 4 == k)
            def _():
                b_unit(i, k, s)
        @pl.when(i % 16 == 15)
        def _():
            with SC('outproj'):
                out_proj(i // 16)
        return c
    def body_m(s, c):
        for k in range(4):
            b_unit(4 * s + k, k, s)
        @pl.when(s % 4 == 3)
        def _():
            with SC('outproj'):
                out_proj(s // 4)
        return c
    def body2(j, c):
        i = first2 + 2 * j
        bufs = ((sB, mB, sA, mA), (sA, mA, sB, mB))
        sep(lambda: stage(i, *bufs[first2 % 2]))
        sep(lambda: stage(i + 1, *bufs[(first2 + 1) % 2]))
        return c
    def pair(i, gen, total, sp, mmf=None):
        pmp = Pump(gen, total)
        stage(i, sB, mB, sA, mA, pump=pmp, span=(0.0, 0.5), speed=sp, mmf=mmf)
        stage(i + 1, sA, mA, sB, mB, pump=pmp, span=(0.5, 1.0), speed=sp, mmf=mmf)
    mmf_of = lambda k, d: (E(k, d)[0] == "1", E(k, d)[1] == "1", int(E(k, d)[2]))
    with SC('loop'):
        if LAY == "d":
            mk = lambda f: (lambda *its: mix(*its)) if f else (lambda *its: chain(*[g for g, _ in its]))
            combA, combB = mk(E("MIXA", "1") == "1"), mk(E("MIXB", "0") == "1")
            OPIN = E("OPIN", "1") == "1"
            def blkA(s, op=False):
                d_ = dict(G=(b_kgen(s, 0, 16), 16 * G_PAIR), C=(b_conv(0, 16), conv_cost(0, 16)))
                its = [d_[k] for k in E("ORDA", "GC")]
                if op:
                    def scaled(gen, f):
                        for kind, cost in gen:
                            yield kind, cost * f
                    its.append((scaled(out_proj_items((s >> 2) - 1), int(E("OPS", "1000"))), 4 * int(E("OPS", "1000"))))
                pair(4 * s, combA(*its), sum(t for _, t in its), float(E("SPA0" if op else "SPA", "1.15")), mmf_of("MA0" if op else "MA", "102"))
            def blkB(s):
                d_ = dict(F=(b_dft(s), int(E("CF", "1500"))), I=(b_inv(s - 1), int(E("CI", "400"))), T=(b_tables(s + 1, 0, 4), 4 * T_OCT))
                its = [d_[k] for k in E("ORDB", "FIT")]
                pair(4 * s + 2, combB(*its), sum(t for _, t in its), float(E("SPB", "1.15")), mmf_of("MB", "111"))
                if not OPIN:
                    @pl.when(s % 4 == 3)
                    def _():
                        out_proj(s // 4)
            def body_d(j, c):
                s = j >> 1
                if OPIN:
                    ev = lambda: lax.cond(((s & 3) == 0) & (s > 0), lambda: blkA(s, True), lambda: blkA(s))
                else:
                    ev = lambda: blkA(s)
                lax.cond((j & 1) == 0, ev, lambda: blkB(s))
                return c
            if E("BRD", "1") == "1":
                lax.fori_loop(0, 2 * NSL, body_d, 0)
            else:
                def body_dm(s, c):
                    blkA(s)
                    blkB(s)
                    return c
                lax.fori_loop(0, NSL, body_dm, 0)
        elif E('BR', '1') == '1':
            lax.fori_loop(0, 4 * NSL, body_s, 0)
        elif E('BR', '1') == '3':
            def body_c(i, c):
                s = i // 4
                def k3():
                    b_unit(i, 3, s)
                    @pl.when(s % 4 == 3)
                    def _():
                        out_proj(s // 4)
                lax.cond(i % 4 < 2,
                         lambda: lax.cond(i % 2 == 0, lambda: b_unit(i, 0, s), lambda: b_unit(i, 1, s)),
                         lambda: lax.cond(i % 2 == 0, lambda: b_unit(i, 2, s), k3))
                return c
            lax.fori_loop(0, 4 * NSL, body_c, 0)
        else:
            lax.fori_loop(0, NSL, body_m, 0)
        i0 = 4 * NSL
        for _d in range(int(E('DUMMY', '0'))):
            lax.fori_loop(0, zz, lambda _, c: (stage(7 + _d, sB, mB, sA, mA), c)[1], 0)
        bufs = lambda i: (sB, mB, sA, mA) if i % 2 == 0 else (sA, mA, sB, mB)
        def once(f):
            if E("ONCE", "1") == "1":
                lax.fori_loop(0, 1 + zz, lambda _, c: (f(), c)[1], 0)
            else:
                pl.when(zz == 0)(f)
        once(lambda: pair(i0, chain(b_conv(0, 16)), conv_cost(0, 16), float(E("SPC", "2.0"))) if E("PP", "0") == "1" else
             stage(i0, *bufs(i0), bwork=(b_conv(0, 16), conv_cost(0, 16)), speed=float(E("SPC", "1.1"))))
        once(lambda: stage(i0 + 1, *bufs(i0 + 1), bwork=(b_inv(NSL - 1), 400), speed=float(E("SPI", "1.5"))))
        once(lambda: stage(i0 + 2, *bufs(i0 + 2), bwork=(finish_b(), S // 128), speed=float(E("SPF", "1.3"))))
        first2 = i0 + 3
        for qb in range(3):
            out_copy(qb).start()
        lastb_copy().start()
        n2 = int(E('N2', '2'))
        if n2 == 1:
            once(lambda: body2(0, 0))
        elif n2 > 1:
            lax.fori_loop(0, n2, body2, 0)
        for i in range(first2 + 2 * n2, n_units - 1):
            stage(i, *bufs(i))
        stage(n_units - 1, None, None, sB, mB, do_q=False, bwork=(out_proj_partial(), NQ // 128), speed=1.5)
    with SC('tail'):
        wlast = upk(wop_ref[192:256, :])
        for c in range(NLC):
            for rb in range(c * LC // 128, (c + 1) * LC // 128):
                cs = slice(QL + 128 * rb, QL + 128 * (rb + 1))
                if OPT:
                    oat = opt_ref[:, 128 * rb:128 * (rb + 1)] + jnp.dot(upk(wopt_ref[...])[:, 384:512], ot_ref[384:512, cs], preferred_element_type=f32)
                    oat = jnp.concatenate([oat, jnp.zeros((64, 128), f32)], axis=0).astype(bf16)
                    ost_ref[cs, 0:448] = oat.T[:, 0:448]
                else:
                    oa = opart_ref[128 * rb:128 * (rb + 1), :] + lax.dot_general(ot_ref[384:512, cs], wlast, TN, preferred_element_type=f32)
                    ost_ref[cs, 0:448] = oa.astype(bf16)
            last_copy(c).start()
        for qb in range(3):
            out_copy(qb).wait()
        lastb_copy().wait()
        for c in range(NLC):
            last_copy(c).wait()


@jax.jit
def pallas_concat_heads__mha_block__ssm_conv_s4__prompt_kernel(A_x, A_wqkv, A_wo, B_u, B_A_re, B_A_im, B_B_re, B_B_im, B_C_re, B_C_im, B_log_dt, B_Dskip):
    V = pltpu.VMEM
    FW = 384 if CFG["g3"] else 256
    TD = D if E("TPRO", "0") == "1" else SL
    scratch = [
        V((D,), bf16), V((D,), bf16), V((D, S), bf16), V((D, 3 * D), bf16), V((D, D), bf16), V((D, S), bf16), V((6, D, N), bf16),
        V((128, 256), bf16), V((256, 128), bf16), V((6, 128, 256), bf16), V((S, 2 * D), bf16),
        V((704, 512), i32), V((3, 256, 512), i32), V((256, D), i32),
        V((16, 64, S), i32), V((4, S // 2, 128), i32), V((256, S), i32),
        V((S, NQ), f32), V((S, NQ), f32), V((8, NQ), f32), V((8, NQ), f32), V((512, S), bf16),
        V((2, D, 128), f32),
        V((4, 8 * TD, 128), i32), V((4, 8 * TD, 128), f32), V((4, TD, 128), f32),
        V((2, 8 * (SL // 2), 128), f32),
        V((16, SL, FW), f32), V((16, SL, FW), f32),
        V((512, S), bf16), V((16 * SL, 256), f32), V((NQ, D), f32), V((D, NQ), f32), V((D // 2, 512), i32),
        pltpu.SemaphoreType.DMA((20,)), pltpu.SemaphoreType.DMA((12,)),
    ]
    anyspec = pl.BlockSpec(memory_space=pl.ANY)
    vspec = pl.BlockSpec(memory_space=pltpu.VMEM)
    out = pl.pallas_call(
        kernel,
        out_shape=jax.ShapeDtypeStruct((S, 2 * D), bf16),
        in_specs=[pl.BlockSpec(memory_space=pltpu.SMEM)] + [anyspec] * 15,
        out_specs=anyspec,
        scratch_shapes=scratch,
        compiler_params=pltpu.CompilerParams(vmem_limit_bytes=124 * 1024 * 1024, flags=FLAGS or None),
    )(np.zeros((1,), np.int32), A_x.reshape(S, D).T, A_wqkv, A_wo, B_u.reshape(S, D).T, B_A_re, B_A_im, B_B_re, B_B_im, B_C_re, B_C_im, B_log_dt, B_Dskip,
      C_FT, C_FINVT, C_GT)
    return out.reshape(1, S, 2 * D)
```

```python
import numpy as np
import jax
import jax.numpy as jnp
from jax import lax
import jax.experimental.pallas as pl
import jax.experimental.pallas.tpu as pltpu
import ml_dtypes

S, D, DH, N = 2048, 448, 28, 256
NQ = 512
R = 128
SL = 32
NSL = D // SL
NCB = 4
CB = S // NCB
N_UNITS = 16 * (S // NQ)
QL = S - NQ
NT = (((1,), (1,)), ((), ()))
f32, bf16, i32 = jnp.float32, jnp.bfloat16, jnp.int32
LOG2E = 1.4426950408889634


def _round_bf16(l):
    u = np.asarray(l, np.float32).view(np.uint32).astype(np.uint64)
    u = (u + 0x7FFF + ((u >> 16) & 1)) & 0xFFFF0000
    return u.astype(np.uint32).view(np.float32).astype(np.int64)


_HI = np.array([0, 1, 2, 3, 4, 5, 6, 7, 512, 516, 1024, 1536, 640, 1152, 1664, 0])


def _dft_consts():
    T, M = 128, 256
    forder = np.concatenate([np.arange(0, T, 2), np.arange(1, T, 2)])
    ang = 2 * np.pi * (forder[:, None] + 0.5) * np.arange(T)[None, :] / M
    F = np.concatenate([np.cos(ang), -np.sin(ang)], 0)
    Finv = np.concatenate([np.cos(ang).T, -np.sin(ang).T], 1) * (2.0 / M)

    def lag_of(upper, blk):
        r = np.arange(8)[:, None] + (8 if upper else 0)
        b = 16 * blk + np.arange(16)[None, :]
        return (_HI[r] + 8 * b).reshape(-1)

    plan, Gs = [], []
    for m in range(16):
        tgt = _round_bf16(T * m + np.arange(T))
        if m < 4:
            cand = [(0, m)] + ([(0, m + 1)] if m == 2 else []) + ([(1, 0)] if m == 3 else [])
        else:
            cand = [(1, m % 4)]
        used = np.zeros(T, bool)
        for (up, blk) in cand:
            lg = lag_of(up, blk)
            valid = np.ones(128, bool)
            if up:
                valid[7 * 16:] = False
            E = np.zeros((T, 128))
            for j in range(T):
                idx = np.where((lg == tgt[j]) & valid)[0]
                if not used[j] and len(idx):
                    E[j, idx[0]] = 1
                    used[j] = True
            Gm = F @ E
            gi = next((k for k, g0 in enumerate(Gs) if np.array_equal(g0, Gm)), None)
            if gi is None:
                Gs.append(Gm)
                gi = len(Gs) - 1
            plan.append((m, up, blk, gi))
        assert used.all()
    return F, Finv, np.stack(Gs), plan


_F, _FINV, _G, _PLAN = _dft_consts()
_np_bf16 = lambda a: np.asarray(a, np.float32).astype(ml_dtypes.bfloat16)
_C_FT = _np_bf16(_F.T)
_C_FINVT = _np_bf16(_FINV.T)
_C_GT = _np_bf16(np.transpose(_G, (0, 2, 1)))


def pk(x):
    return pltpu.bitcast(x, i32)


def upk(x):
    return pltpu.bitcast(x, bf16)


def cmul(ar, ai, br, bi):
    return ar * br - ai * bi, ar * bi + ai * br


def fold8(t):
    sub = lax.broadcasted_iota(jnp.int32, (8, 128), 0)
    seg = lax.broadcasted_iota(jnp.int32, (8, 128), 1) >> 4
    for k in (4, 2, 1):
        sb = (sub & k) != 0
        gb = (seg & k) != 0
        up = pltpu.roll(pltpu.roll(t, 8 - k, 0), 16 * k, 1)
        dn = pltpu.roll(pltpu.roll(t, k, 0), 128 - 16 * k, 1)
        t = jnp.where(sb == gb, t, jnp.where(gb, up, dn))
    return t


def sub_transpose8(xs):
    xs = list(xs)
    sub = lax.broadcasted_iota(jnp.int32, (8, 128), 0)
    for k in (4, 2, 1):
        keep = (sub & k) == 0
        new = list(xs)
        for a in range(8):
            if a & k:
                continue
            b = a ^ k
            new[a] = jnp.where(keep, xs[a], pltpu.roll(xs[b], k, 0))
            new[b] = jnp.where(keep, pltpu.roll(xs[a], 8 - k, 0), xs[b])
        xs = new
    return xs


class Pump:
    def __init__(self, gen, total):
        self.gen, self.total, self.done = gen, total, 0.0
        self.pending = next(gen, None) if gen is not None else None

    def to(self, frac, mm=True, max_mm=99):
        n_mm = 0
        while self.pending is not None and self.done < frac * self.total - 1e-9:
            kind, cost = self.pending
            if kind == "m":
                if not mm or n_mm >= max_mm:
                    break
                n_mm += 1
            self.done += cost
            self.pending = next(self.gen, None)

    def finish(self):
        while self.pending is not None:
            self.pending = next(self.gen, None)


def chain(*gens):
    for g in gens:
        yield from g


def mix(*items):
    st = [[g, float(t), 0.0, next(g, None)] for g, t in items]
    while True:
        live = [x for x in st if x[3] is not None]
        if not live:
            return
        x = min(live, key=lambda y: y[2] / y[1])
        kind, cost = x[3]
        yield kind, cost
        x[2] += cost
        x[3] = next(x[0], None)


def scaled(gen, f):
    for kind, cost in gen:
        yield kind, cost * f


def _kernel(z_ref, xt_hbm, wqkv_hbm, wo_hbm, ut_hbm, are_hbm, aim_hbm, bre_hbm, bim_hbm, cre_hbm, cim_hbm,
            ldt_hbm, dsk_hbm, FT_hbm, FinvT_hbm, GT_hbm,
            out_hbm,
            ldt_ref, dsk_ref, xt_ref, wqkv_ref, wo_ref, uin_ref, par_ref, FT_ref, FinvT_ref, GT_ref, ost_ref,
            wt_ref, wp_ref, wop_ref, wopt_ref, qm_ref, k_ref, vt_ref, sA, sB, mA, mB, ot_ref,
            col_ref, a_tab, v0_tab, y8_tab, kt_ref, bm_ref, ut_ref, yt_ref, yh_ref, opt_ref, sem_in, sem_out):
    zz = z_ref[0]

    par_hbm = (are_hbm, aim_hbm, bre_hbm, bim_hbm, cre_hbm, cim_hbm)
    cp_w = [pltpu.make_async_copy(wqkv_hbm.at[:, pl.ds(a, n)], wqkv_ref.at[:, pl.ds(a, n)], sem_in.at[k])
            for k, (a, n) in enumerate(((384, 512), (896, 448), (0, 384)))]
    cp_x = [pltpu.make_async_copy(xt_hbm.at[:, pl.ds(cb * CB, CB)], xt_ref.at[:, pl.ds(cb * CB, CB)], sem_in.at[3 + cb])
            for cb in range(NCB)]
    cp_p = [pltpu.make_async_copy(par_hbm[k], par_ref.at[k], sem_in.at[7 + k]) for k in range(6)]
    cp_wo = pltpu.make_async_copy(wo_hbm, wo_ref, sem_in.at[13])
    cp_c = [pltpu.make_async_copy(a, b, sem_in.at[14 + k])
            for k, (a, b) in enumerate(((FT_hbm, FT_ref), (FinvT_hbm, FinvT_ref), (GT_hbm, GT_ref)))]
    cp_u = pltpu.make_async_copy(ut_hbm, uin_ref, sem_in.at[17])
    cp_v = [pltpu.make_async_copy(ldt_hbm, ldt_ref, sem_in.at[18]), pltpu.make_async_copy(dsk_hbm, dsk_ref, sem_in.at[19])]
    for cp in [cp_w[0], cp_x[0], cp_w[1], cp_x[1], cp_w[2]] + cp_x[2:] + [cp_wo] + cp_v + cp_p + cp_c + [cp_u]:
        cp.start()

    yt_ref[0:64, :] = jnp.zeros((64, S), bf16)
    yh_ref[...] = jnp.zeros(yh_ref.shape, f32)

    def w_transpose(tiles):
        for c in tiles:
            c1 = min(128 * (c + 1), 3 * D)
            blk = wqkv_ref[:, 128 * c:c1]
            blk = jnp.concatenate([blk, jnp.zeros((512 - D, c1 - 128 * c), bf16)], axis=0)
            if c1 - 128 * c < 128:
                blk = jnp.concatenate([blk, jnp.zeros((512, 128 - (c1 - 128 * c)), bf16)], axis=1)
            wt_ref[64 * c:64 * (c + 1), :] = pk(blk.T)

    def w_respace(part, hs=range(16)):
        z2 = jnp.zeros((2, 512), i32)
        for h in hs:
            r0 = (D * part + DH * h) // 2
            wp_ref[part, 16 * h:16 * (h + 1), :] = jnp.concatenate([wt_ref[r0:r0 + 14, :], z2], axis=0)

    def w_prep(tiles, part):
        for c in tiles:
            yield "v", 2
            w_transpose((c,))
        for h in range(0, 16, 4):
            yield "v", 1
            w_respace(part, range(h, h + 4))

    def late_prep():
        yield "v", 6
        ldt = ldt_ref[...].astype(f32).reshape(1, D)
        dsk = dsk_ref[...].astype(f32).reshape(1, D)
        dt_row = jnp.exp(ldt).astype(bf16).astype(f32)
        col_ref[0] = jnp.broadcast_to(dt_row, (128, D)).T
        col_ref[1] = jnp.broadcast_to(dsk, (128, D)).T
        wo = pk(wo_ref[...])
        z2 = jnp.zeros((2, D), i32)
        for h in range(16):
            if h % 4 == 0:
                yield "v", 1
            wop_ref[16 * h:16 * (h + 1), :] = jnp.concatenate([wo[14 * h:14 * h + 14], z2], axis=0)

    def wopt_prep():
        for c in range(4):
            yield "v", 1
            blk = jnp.concatenate([upk(wop_ref[64 * c:64 * (c + 1), :]), jnp.zeros((128, 64), bf16)], axis=1)
            wopt_ref[:, 128 * c:128 * (c + 1)] = pk(blk.T[0:D, :])

    def b_tables(s):
        s = min(s, NSL - 1) if isinstance(s, int) else jnp.minimum(s, NSL - 1)
        d0 = s * SL if isinstance(s, int) else pl.multiple_of(s * SL, SL)
        trow = lambda v, c: slice((8 * v + c) * 8, (8 * v + c) * 8 + 8)
        for v in range(SL // 8):
            rs = pl.ds(pl.multiple_of(d0 + 8 * v, 8), 8)
            dt = col_ref[0, rs, :]
            for t in range(2):
                ls = slice(128 * t, 128 * (t + 1))
                ld = lambda k: par_ref[k, rs, ls].astype(f32)
                yield "v", 100
                a_re, a_im = dt * ld(0), dt * ld(1)
                mag = jnp.exp(a_re)
                zr = mag * jnp.cos(a_im)
                yield "v", 60
                z = (zr, mag * jnp.sin(a_im))
                yield "v", 60
                z2 = cmul(*z, *z)
                z4 = cmul(*z2, *z2)
                y = cmul(*z4, *z4)
                rows = [(jnp.ones_like(zr), jnp.zeros_like(zr)), y]
                for r in range(6):
                    rows.append(cmul(*rows[-1], *y))
                yield "v", 70
                tr = sub_transpose8([x[0] for x in rows])
                for c in range(8):
                    v0_tab[t, trow(v, c), :] = tr[c]
                yield "v", 70
                ti = sub_transpose8([x[1] for x in rows])
                for c in range(8):
                    v0_tab[2 + t, trow(v, c), :] = ti[c]
                yield "v", 40
                z16 = cmul(*y, *y)
                z32 = cmul(*z16, *z16)
                z64 = cmul(*z32, *z32)
                y8_tab[t, 8 * v:8 * v + 8, :] = z64[0]
                y8_tab[2 + t, 8 * v:8 * v + 8, :] = z64[1]
                z128 = cmul(*z64, *z64)
                z256 = cmul(*z128, *z128)
                z512 = cmul(*z256, *z256)
                wr, wi = [], []

                def put_pair(x0, x1):
                    wr.append(pltpu.pack_elementwise([x0[0], x1[0]], packed_dtype=bf16))
                    wi.append(pltpu.pack_elementwise([-x0[1], -x1[1]], packed_dtype=bf16))
                yield "v", 40
                w = cmul(ld(4), ld(5), dt * ld(2), dt * ld(3))
                cur = w
                for j in range(4):
                    nxt = cmul(*cur, *z)
                    put_pair(cur, nxt)
                    if j < 3:
                        cur = cmul(*nxt, *z)
                    if j == 1:
                        yield "v", 30
                yield "v", 50
                w512 = cmul(*w, *z512)
                put_pair(w512, cmul(*w512, *z4))
                w1024 = cmul(*w512, *z512)
                w1536 = cmul(*w1024, *z512)
                put_pair(w1024, w1536)
                put_pair(cmul(*w512, *z128), cmul(*w1024, *z128))
                zero = jnp.zeros_like(zr)
                put_pair(cmul(*w1536, *z128), (zero, zero))
                yield "v", 75
                tr = sub_transpose8(wr)
                for c in range(8):
                    a_tab[t, trow(v, c), :] = tr[c]
                yield "v", 75
                ti = sub_transpose8(wi)
                for c in range(8):
                    a_tab[2 + t, trow(v, c), :] = ti[c]
    T_COST = 4 * 2 * 680

    scale = (DH ** -0.5) * LOG2E
    tpump, tcount = [None], [0]

    def proj(part, cb, gs=range(4)):
        c0 = cb * CB
        cs = slice(c0, c0 + CB)
        xt = xt_ref[:, cs]
        rows = lax.broadcasted_iota(jnp.int32, (128, CB), 0)
        for g in gs:
            o = jnp.dot(upk(wp_ref[part, 64 * g:64 * (g + 1), :])[:, 0:D], xt, preferred_element_type=f32)
            if part == 1:
                k_ref[g, c0 // 2:(c0 + CB) // 2, :] = pk(o.astype(bf16).T)
            elif part == 2:
                vt_ref[64 * g:64 * (g + 1), cs] = pk(jnp.where((rows & 31) == 28, 1.0, o).astype(bf16))
            else:
                q = o * scale
                for hh in range(4):
                    qm_ref[4 * g + hh, :, cs] = pk(jnp.where((rows >> 5) == hh, q, 0.0).astype(bf16))
            if tpump[0] is not None:
                tcount[0] += 1
                tpump[0].to(tcount[0] / 17)

    cp_w[0].wait()
    w_transpose((3, 4, 5, 6))
    w_respace(1)
    cp_x[0].wait()
    proj(1, 0, (0, 1, 2))
    cp_w[1].wait()
    wpump = Pump(w_prep((7, 8, 9, 10), 2), 12)
    wpump.to(0.999)
    proj(1, 0, (3,))
    wpump.finish()
    proj(2, 0)
    cp_x[1].wait()
    cp_w[2].wait()
    wpump = Pump(w_prep((0, 1, 2), 0), 10)
    for g in range(4):
        wpump.to((g + 1) / 3 * 0.999)
        proj(1, 1, (g,))
    wpump.finish()
    proj(2, 1)
    proj(0, 0)
    proj(0, 1)
    for cp in [cp_x[2], cp_x[3], cp_wo] + cp_v + cp_p:
        cp.wait()
    lpump = Pump(late_prep(), 10)
    for g in range(4):
        lpump.to((g + 1) / 3 * 0.999)
        proj(1, 2, (g,))
    lpump.finish()
    tpump[0] = Pump(b_tables(0), T_COST)
    for part, cb in ((2, 2), (0, 2), (1, 3), (2, 3), (0, 3)):
        proj(part, cb)
    tpump[0].finish()

    def b_kgen():
        lane = lax.broadcasted_iota(jnp.int32, (8, 128), 1)
        HP = SL // 2
        for g in range(HP):
            o = None
            for t in range(2):
                re, im = [], []
                for ch in range(2):
                    d = g + HP * ch
                    yield "v", 50
                    vr, vi = v0_tab[t, 8 * d:8 * d + 8, :], v0_tab[2 + t, 8 * d:8 * d + 8, :]
                    mr = jnp.broadcast_to(y8_tab[t, d:d + 1, :], (8, 128))
                    mi = jnp.broadcast_to(y8_tab[2 + t, d:d + 1, :], (8, 128))
                    rr, ii = [vr], [vi]
                    for j in range(7):
                        nr, ni = cmul(rr[-1], ii[-1], mr, mi)
                        rr.append(nr)
                        ii.append(ni)
                    re.extend(rr)
                    im.extend(ii)
                yield "m", 20
                for kt, rhs in ((t, re), (2 + t, im)):
                    A = jnp.concatenate([upk(a_tab[kt, 8 * (g + HP * ch):8 * (g + HP * ch) + 8, :]) for ch in range(2)], axis=0)
                    dd = lax.dot_general(A, jnp.concatenate(rhs, axis=0).astype(bf16), NT, preferred_element_type=f32)
                    o = dd if o is None else o + dd
            yield "v", 40
            kt_ref[0, 8 * g:8 * (g + 1), :] = fold8(jnp.where(lane < 64, o[0:8], o[16:24]))
            kt_ref[1, 8 * g:8 * (g + 1), :] = fold8(jnp.where(lane < 64, o[8:16], o[24:32]))
    G_COST = (SL // 2) * 280

    def put_b(m, c, d):
        bm_ref[m, :, 0:128] = c
        bm_ref[m, :, 128:256] = d - c
        bm_ref[m, :, 256:384] = c + d

    def put_u(j, a, b):
        ut_ref[j, :, 0:128] = a + b
        ut_ref[j, :, 128:256] = a
        ut_ref[j, :, 256:384] = b

    def b_dft(s):
        d0 = pl.multiple_of(jnp.minimum(s, NSL - 1) * SL, SL)
        HP = SL // 2
        prev = None
        sgn = jnp.where(lax.broadcasted_iota(jnp.int32, (SL, 128), 1) < 64, 1.0, -1.0)
        for jb in range(4):
            yield "m", 120
            lhs = jnp.concatenate([uin_ref[pl.ds(d0, SL), 128 * j:128 * (j + 1)] for j in range(4 * jb, 4 * jb + 4)], axis=0)
            o = jnp.dot(lhs, FT_ref[...], preferred_element_type=f32)
            for k in range(4):
                ur, ui = o[k * SL:(k + 1) * SL, 0:128], o[k * SL:(k + 1) * SL, 128:256]
                if prev is None:
                    put_u(4 * jb + k, ur, ui)
                else:
                    put_u(4 * jb + k, ur - sgn * prev[1], ui + sgn * prev[0])
                prev = (ur, ui)
        tiles = {}
        for up in range(2):
            yield "v", 150
            for blk in range(4):
                parts = [kt_ref[up, pl.ds(ch * 4 + blk, HP, stride=8), :] for ch in range(2)]
                tiles[(up, blk)] = jnp.concatenate(parts, axis=0).astype(bf16)
        by_g = {}
        for (m, up, blk, gi) in _PLAN:
            by_g.setdefault(gi, []).append((m, up, blk))
        res = {}
        dcol = col_ref[1, pl.ds(d0, SL), :]
        for gi in range(6):
            yield "m", 120
            lst = by_g[gi]
            lhs = jnp.concatenate([tiles[(up, blk)] for (_, up, blk) in lst], axis=0)
            o = jnp.dot(lhs, GT_ref[gi], preferred_element_type=f32)
            for k, (m, _, _) in enumerate(lst):
                piece = o[k * SL:(k + 1) * SL]
                res[m] = piece if m not in res else res[m] + piece
            if gi == 1:
                continue
            for m in sorted(set(x[0] for x in lst)):
                vr, vi = res[m][:, 0:128], res[m][:, 128:256]
                if m == 0:
                    vr = vr + dcol
                put_b(m, vr, vi)
    F_COST = 1500

    def b_conv():
        for i in range(16):
            for v in range(SL // 8):
                rs = slice(8 * v, 8 * (v + 1))
                a1 = a2 = a3 = None
                for m in range(i + 1):
                    if m % 2 == 0:
                        yield "v", 8 * min(2, i + 1 - m)
                    j = i - m
                    p1 = bm_ref[m, rs, 0:128] * ut_ref[j, rs, 0:128]
                    p2 = bm_ref[m, rs, 128:256] * ut_ref[j, rs, 128:256]
                    p3 = bm_ref[m, rs, 256:384] * ut_ref[j, rs, 256:384]
                    a3 = p3 if a3 is None else a3 + p3
                    a1 = p1 if a1 is None else a1 + p1
                    a2 = p2 if a2 is None else a2 + p2
                yr, yi = a1 - a3, a1 + a2
                yh_ref[i * SL + 8 * v:i * SL + 8 * (v + 1), 0:128] = yr
                yh_ref[i * SL + 8 * v:i * SL + 8 * (v + 1), 128:256] = yi
    C_COST = sum(32 * (i + 1) for i in range(16))

    def b_inv(s):
        r0 = pl.multiple_of(64 + s * SL, SL)
        for ib in range(4):
            yield "m", 100
            lhs = yh_ref[4 * SL * ib:4 * SL * (ib + 1), :].astype(bf16)
            o = jnp.dot(lhs, FinvT_ref[...], preferred_element_type=f32)
            for k in range(4):
                i = 4 * ib + k
                yt_ref[pl.ds(r0, SL), 128 * i:128 * (i + 1)] = o[k * SL:(k + 1) * SL].astype(bf16)
    I_COST = 400

    def finish_b():
        for tb in range(S // 128):
            yield "v", 1
            rs = slice(128 * tb, 128 * (tb + 1))
            yb = yt_ref[:, rs].T
            ost_ref[rs, 448:896] = yb[:, 64:512]

    def stage(i, s_new, m_new, s_old, m_old, do_q=True, do_e=True, pump=None, span=(0.0, 1.0), speed=1.0,
              mmf=(True, False, 1)):
        nchunk = S // R
        if pump is None:
            pump = Pump(None, 0)
        prog = lambda x: speed * (span[0] + (span[1] - span[0]) * x)
        m1, m2, mx = mmf
        if do_e:
            h = i & 15
            q0 = pl.multiple_of((i >> 4) * NQ, NQ)
            r0 = pl.multiple_of(h * 16, 16)
            mo = jnp.max(m_old[...], axis=0, keepdims=True)
        if do_q:
            hq = (i + 1) & 15
            qq0 = pl.multiple_of((((i + 1) >> 4) & 3) * NQ, NQ)
            h4 = hq >> 2
            qm = upk(qm_ref[hq, :, pl.ds(qq0, NQ)])
        mrun = None
        acc = None
        for c in range(nchunk):
            rs = slice(c * R, (c + 1) * R)
            last = do_q and do_e and c == nchunk - 1 and span[1] == 1.0
            if do_q and not last:
                s = jnp.dot(upk(k_ref[h4, c * R // 2:(c + 1) * R // 2, :]), qm, preferred_element_type=f32)
            if do_e:
                p = jnp.exp2(s_old[rs, :] - mo).astype(bf16)
            if last:
                dd = jnp.dot(upk(vt_ref[pl.ds(r0, 16), rs]), p, preferred_element_type=f32)
                acc = dd if acc is None else acc + dd
                s = jnp.dot(upk(k_ref[h4, c * R // 2:(c + 1) * R // 2, :]), qm, preferred_element_type=f32)
            pump.to(prog((2 * c + 1) / (2 * nchunk)), mm=m1, max_mm=mx)
            if do_q:
                s_new[rs, :] = s
                mc = jnp.max(s.reshape(R // 8, 8, NQ), axis=0)
                mrun = mc if mrun is None else jnp.maximum(mrun, mc)
            if do_e and not last:
                dd = jnp.dot(upk(vt_ref[pl.ds(r0, 16), rs]), p, preferred_element_type=f32)
                acc = dd if acc is None else acc + dd
            pump.to(prog((2 * c + 2) / (2 * nchunk)), mm=m2, max_mm=mx)
        if span[1] == 1.0:
            pump.finish()
        if do_q:
            m_new[...] = mrun
        if do_e:
            o = acc / acc[28:29, :]
            ot_ref[pl.ds(pl.multiple_of(h * 32, 32), 32), pl.ds(q0, NQ)] = o.astype(bf16)

    def bufs(i):
        return (sB, mB, sA, mA) if i % 2 == 0 else (sA, mA, sB, mB)

    def pair(i, gen, total, speed, mmf=(True, False, 1)):
        pump = Pump(gen, total)
        stage(i, *bufs(0), pump=pump, span=(0.0, 0.5), speed=speed, mmf=mmf)
        stage(i + 1, *bufs(1), pump=pump, span=(0.5, 1.0), speed=speed, mmf=mmf)

    def store_oa(cs, oat):
        oat = jnp.concatenate([oat, jnp.zeros((64, 128), f32)], axis=0).astype(bf16)
        ost_ref[cs, 0:D] = oat.T[:, 0:D]

    def out_proj_items(qb):
        q0 = pl.multiple_of(qb * NQ, NQ)
        for rb in range(NQ // 128):
            yield "m", 1
            cs = pl.ds(q0 + 128 * rb, 128)
            store_oa(cs, jnp.dot(upk(wopt_ref[...]), ot_ref[:, cs], preferred_element_type=f32))

    def out_proj_partial():
        for rb in range(NQ // 128):
            yield "m", 1
            cs = slice(QL + 128 * rb, QL + 128 * (rb + 1))
            opt_ref[:, 128 * rb:128 * (rb + 1)] = jnp.dot(upk(wopt_ref[...])[:, 0:384], ot_ref[0:384, cs],
                                                          preferred_element_type=f32)

    def out_copy(qb):
        return pltpu.make_async_copy(ost_ref.at[pl.ds(qb * NQ, NQ)], out_hbm.at[pl.ds(qb * NQ, NQ)], sem_out.at[qb])

    def lastb_copy():
        return pltpu.make_async_copy(ost_ref.at[pl.ds(QL, NQ), pl.ds(512, 384)],
                                     out_hbm.at[pl.ds(QL, NQ), pl.ds(512, 384)], sem_out.at[3])

    def last_copy(c):
        rows = pl.ds(QL + 128 * c, 128)
        return pltpu.make_async_copy(ost_ref.at[rows, pl.ds(0, 512)], out_hbm.at[rows, pl.ds(0, 512)], sem_out.at[4 + c])

    def once(f):
        lax.fori_loop(0, 1 + zz, lambda _, c: (f(), c)[1], 0)

    bm_ref[...] = jnp.zeros(bm_ref.shape, f32)
    ut_ref[...] = jnp.zeros(ut_ref.shape, f32)
    stage(-1, sA, mA, None, None, do_e=False, pump=Pump(wopt_prep(), 4), speed=1.4)
    for cp in cp_c + [cp_u]:
        cp.wait()

    def block_a(s, op=False):
        its = [(b_conv(), C_COST), (b_kgen(), G_COST)]
        if op:
            its.append((scaled(out_proj_items((s >> 2) - 1), 100), 400))
        pair(4 * s, mix(*its), sum(t for _, t in its), 1.2 if op else 1.25, (True, False, 2))

    def block_b(s):
        pair(4 * s + 2, chain(b_tables(s + 1), b_inv(s - 1), b_dft(s)), T_COST + I_COST + F_COST, 0.97, (True, True, 1))

    def body(j, c):
        s = j >> 1
        lax.cond((j & 1) == 0,
                 lambda: lax.cond(((s & 3) == 0) & (s > 0), lambda: block_a(s, True), lambda: block_a(s)),
                 lambda: block_b(s))
        return c
    lax.fori_loop(0, 2 * NSL, body, 0)

    i0 = 4 * NSL
    once(lambda: stage(i0, *bufs(i0), pump=Pump(b_conv(), C_COST), speed=1.0))

    def drain_b():
        pump = Pump(chain(b_inv(NSL - 1), scaled(finish_b(), 25)), 800)
        stage(i0 + 1, *bufs(i0 + 1), pump=pump, span=(0.0, 0.5), speed=1.1)
        stage(i0 + 2, *bufs(i0 + 2), pump=pump, span=(0.5, 1.0), speed=1.1)
    once(drain_b)
    for qb in range(3):
        out_copy(qb).start()
    lastb_copy().start()

    def plain_pair(j, c):
        i = i0 + 3 + 2 * j
        stage(i, *bufs(i0 + 3))
        stage(i + 1, *bufs(i0 + 4))
        return c
    lax.fori_loop(0, 2, plain_pair, 0)
    stage(N_UNITS - 1, None, None, sB, mB, do_q=False, pump=Pump(out_proj_partial(), NQ // 128), speed=1.5)

    for rb in range(NQ // 128):
        cs = slice(QL + 128 * rb, QL + 128 * (rb + 1))
        store_oa(cs, opt_ref[:, 128 * rb:128 * (rb + 1)]
                 + jnp.dot(upk(wopt_ref[...])[:, 384:512], ot_ref[384:512, cs], preferred_element_type=f32))
        last_copy(rb).start()
    for qb in range(3):
        out_copy(qb).wait()
    lastb_copy().wait()
    for c in range(NQ // 128):
        last_copy(c).wait()


@jax.jit
def pallas_concat_heads__mha_block__ssm_conv_s4__prompt_kernel(
    A_x: jax.Array,
    A_wqkv: jax.Array,
    A_wo: jax.Array,
    B_u: jax.Array,
    B_A_re: jax.Array,
    B_A_im: jax.Array,
    B_B_re: jax.Array,
    B_B_im: jax.Array,
    B_C_re: jax.Array,
    B_C_im: jax.Array,
    B_log_dt: jax.Array,
    B_Dskip: jax.Array,
):
    V = pltpu.VMEM
    scratch = [
        V((D,), bf16), V((D,), bf16), V((D, S), bf16), V((D, 3 * D), bf16), V((D, D), bf16), V((D, S), bf16),
        V((6, D, N), bf16), V((128, 256), bf16), V((256, 128), bf16), V((6, 128, 256), bf16), V((S, 2 * D), bf16),
        V((704, 512), i32), V((3, 256, 512), i32), V((256, D), i32), V((D // 2, 512), i32),
        V((16, 64, S), i32), V((4, S // 2, 128), i32), V((256, S), i32),
        V((S, NQ), f32), V((S, NQ), f32), V((8, NQ), f32), V((8, NQ), f32), V((512, S), bf16),
        V((2, D, 128), f32),
        V((4, 8 * SL, 128), i32), V((4, 8 * SL, 128), f32), V((4, SL, 128), f32),
        V((2, 8 * (SL // 2), 128), f32),
        V((16, SL, 384), f32), V((16, SL, 384), f32),
        V((512, S), bf16), V((16 * SL, 256), f32), V((D, NQ), f32),
        pltpu.SemaphoreType.DMA((20,)), pltpu.SemaphoreType.DMA((8,)),
    ]
    hbm = pl.BlockSpec(memory_space=pl.ANY)
    out = pl.pallas_call(
        _kernel,
        out_shape=jax.ShapeDtypeStruct((S, 2 * D), bf16),
        in_specs=[pl.BlockSpec(memory_space=pltpu.SMEM)] + [hbm] * 15,
        out_specs=hbm,
        scratch_shapes=scratch,
        compiler_params=pltpu.CompilerParams(vmem_limit_bytes=124 * 1024 * 1024),
    )(np.zeros((1,), np.int32), A_x.reshape(S, D).T, A_wqkv, A_wo, B_u.reshape(S, D).T,
      B_A_re, B_A_im, B_B_re, B_B_im, B_C_re, B_C_im, B_log_dt, B_Dskip, _C_FT, _C_FINVT, _C_GT)
    return out.reshape(1, S, 2 * D)
```
